```python
import jax
import jax.numpy as jnp

def _softmax(x, axis=-1):
    return jax.nn.softmax(x, axis=axis)
def _gelu(x):
    return jax.nn.gelu(x, approximate=True)
def _silu(x):
    return jax.nn.silu(x)
def _sigmoid(x):
    return jax.nn.sigmoid(x)
def _layernorm(x, axis=-1, eps=1e-5):
    m = jnp.mean(x, axis=axis, keepdims=True)
    v = jnp.var(x, axis=axis, keepdims=True)
    return (x - m) / jnp.sqrt(v + eps)
def _scatter_add(tgt, idx, src, axis=0):
    return tgt.at[idx].add(src)
def _segment_sum(src, seg, n):
    return jax.ops.segment_sum(src, seg, n)
class _Rng:
    def __init__(self, key):
        self._k = key
    def _next(self):
        self._k, sub = jax.random.split(self._k)
        return sub
    def normal(self, shape):
        return jax.random.normal(self._next(), shape, dtype=jnp.bfloat16)
    def randint(self, lo, hi, shape):
        return jax.random.randint(self._next(), shape, lo, hi, dtype=jnp.int32)
    def uniform(self, shape, lo=0.0, hi=1.0):
        return jax.random.uniform(self._next(), shape, jnp.bfloat16, lo, hi)
    def permutation(self, n):
        return jax.random.permutation(self._next(), n)


kernel_name = 'recurrent_scan__sliding_local_dilated__swiglu_ffn__prompt'

def setup_inputs():
    _rng = _Rng(jax.random.key(int.from_bytes(__import__("os").urandom(4), "little")))
    _w = (lambda a: (lambda t: t.astype(jnp.bfloat16) if jnp.issubdtype(t.dtype, jnp.floating) else t)(jnp.asarray(a)))
    def _A_setup():
        B, S, D = 1, 2048, 1024
        return {
            "x": _w((lambda *s: _rng.normal(s) * 0.05)(B, S, D)),
            "wqkv": _w((lambda *s: _rng.normal(s) * 0.05)(D, 3 * D)),
            "wo": _w((lambda *s: _rng.normal(s) * 0.05)(D, D)),
        }
    _A_in = _A_setup()

    def _B_setup():
        B, S, D, F = 1, 2048, 1024, 3584
        return {
            "x": _w((lambda *s: _rng.normal(s) * 0.05)(B, S, D)),
            "w_gate": _w((lambda *s: _rng.normal(s) * 0.05)(D, F)),
            "w_up": _w((lambda *s: _rng.normal(s) * 0.05)(D, F)),
            "w_down": _w((lambda *s: _rng.normal(s) * 0.05)(F, D)),
        }
    _B_in = _B_setup()

    return {
        "A_x": _A_in["x"],
        "A_wqkv": _A_in["wqkv"],
        "A_wo": _A_in["wo"],
        "B_x": _B_in["x"],
        "B_w_gate": _B_in["w_gate"],
        "B_w_up": _B_in["w_up"],
        "B_w_down": _B_in["w_down"],
    }

def reference(A_x, A_wqkv, A_wo, B_x, B_w_gate, B_w_up, B_w_down):
    def _A_ref(x, wqkv, wo):
        B, S, D = x.shape
        H = 32; Dh = D // H
        W, dil = 8, 2
        qkv = (lambda x, *d: x.transpose(*d))((x @ wqkv).reshape(B, S, 3, H, Dh), 2, 0, 3, 1, 4)
        q, k, v = qkv[0], qkv[1], qkv[2]
        scale = Dh ** -0.5
        pos = jnp.arange(S)
        off = jnp.arange(W) * dil
        idx = pos[:, None] - off[None, :]
        mask = idx >= 0
        idx_c = jnp.where(mask, idx, 0).reshape(-1)
        kg = k[:, :, idx_c, :].reshape(B, H, S, W, Dh)
        vg = v[:, :, idx_c, :].reshape(B, H, S, W, Dh)
        logits = jnp.einsum("bhsd,bhswd->bhsw", q, kg) * scale
        logits = jnp.where(mask[None, None, :, :], logits, -1e9)
        attn = _softmax(logits, axis=-1)
        o = jnp.einsum("bhsw,bhswd->bhsd", attn, vg)
        return (lambda x, *d: x.transpose(*d))(o, 0, 2, 1, 3).reshape(B, S, D) @ wo

    def _B_ref(x, w_gate, w_up, w_down):
        g = _silu(x @ w_gate)
        u = x @ w_up
        return (g * u) @ w_down

    x = A_x
    xn = _layernorm(x, axis=-1)
    s = _A_ref(xn, A_wqkv, A_wo)
    g = _silu(_B_ref(xn, B_w_gate, B_w_up, B_w_down))
    return x + s * g
```

```python
import functools
import jax
import jax.numpy as jnp
import numpy as np
from jax import lax
import jax.experimental.pallas as pl
import jax.experimental.pallas.tpu as pltpu

S, D, F, H, DH = 2048, 1024, 3584, 32, 32
W, DIL = 8, 2
HALO = 16
f32, bf16 = jnp.float32, jnp.bfloat16


def _level(a, b, bit, lane):
    lo = (lane & (1 << bit)) == 0
    x = jnp.where(lo, a, b)
    y = jnp.take_along_axis(jnp.where(lo, b, a), lane ^ (1 << bit), axis=1)
    return x, y


def _unlevel(x, y, bit, lane):
    lo = (lane & (1 << bit)) == 0
    yp = jnp.take_along_axis(y, lane ^ (1 << bit), axis=1)
    return jnp.where(lo, x, yp), jnp.where(lo, yp, x)


def twist(c):
    lane = lax.broadcasted_iota(jnp.int32, c[0].shape, 1)
    n = [None] * 8
    for p in range(4):
        n[p], n[4 + p] = _level(c[2 * p], c[2 * p + 1], 4, lane)
    c, n = n, [None] * 8
    for g in range(2):
        for p in range(2):
            n[g * 4 + p], n[g * 4 + 2 + p] = _level(c[g * 4 + 2 * p], c[g * 4 + 2 * p + 1], 3, lane)
    c, n = n, [None] * 8
    for g in range(4):
        n[g * 2], n[g * 2 + 1] = _level(c[g * 2], c[g * 2 + 1], 2, lane)
    return n


def untwist(t):
    lane = lax.broadcasted_iota(jnp.int32, t[0].shape, 1)
    n = [None] * 8
    for g in range(4):
        n[g * 2], n[g * 2 + 1] = _unlevel(t[g * 2], t[g * 2 + 1], 2, lane)
    c, n = n, [None] * 8
    for g in range(2):
        for p in range(2):
            n[g * 4 + 2 * p], n[g * 4 + 2 * p + 1] = _unlevel(c[g * 4 + p], c[g * 4 + 2 + p], 3, lane)
    c, n = n, [None] * 8
    for p in range(4):
        n[2 * p], n[2 * p + 1] = _unlevel(c[p], c[4 + p], 4, lane)
    return n


def _tree_sum(xs):
    xs = list(xs)
    while len(xs) > 1:
        nxt = [xs[i] + xs[i + 1] for i in range(0, len(xs) - 1, 2)]
        if len(xs) % 2:
            nxt.append(xs[-1])
        xs = nxt
    return xs[0]


def make(M=256, FC=512, R=32, peel=True, silu_mode="sig", order="inter", vmem_mb=100, lnpipe=True):
    NT = S // M
    NC = F // FC
    scale = DH ** -0.5

    def silu(g):
        if silu_mode == "sig":
            return g * jax.nn.sigmoid(g)
        if silu_mode == "tanh":
            hg = 0.5 * g
            return hg * jnp.tanh(hg) + hg
        if silu_mode == "rcp":
            return g * pl.reciprocal(1.0 + jnp.exp(-g), approx=True)
        raise ValueError

    def kernel(x_ref, wqkv_h, wo_h, wg_h, wu_h, wd_h, out_ref,
               wqkv_v, wo_v, wg_v, wu_v, wd_v, xn_s, q_s, k_s, v_s, o_s, sems):
        step = pl.program_id(0)

        def cp_qkv(p):
            return pltpu.make_async_copy(wqkv_h.at[:, pl.ds(p * D, D)], wqkv_v.at[:, pl.ds(p * D, D)], sems.at[p])
        rest = [(wg_h, wg_v), (wu_h, wu_v), (wd_h, wd_v), (wo_h, wo_v)]
        def cp_rest(i):
            return pltpu.make_async_copy(rest[i][0], rest[i][1], sems.at[3 + i])

        def layernorm_to(base):
            x = x_ref[...].astype(f32)
            mu = jnp.mean(x, axis=-1, keepdims=True)
            xc = x - mu
            var = jnp.mean(xc * xc, axis=-1, keepdims=True)
            xn_s[pl.ds(base, M), :] = (xc * lax.rsqrt(var + 1e-5)).astype(bf16)

        @pl.when(step == 0)
        def _():
            for p in range(3):
                cp_qkv(p).start()
            for i in range(4):
                cp_rest(i).start()
            k_s[pl.ds(0, HALO), :] = jnp.zeros((HALO, D), f32)
            v_s[pl.ds(0, HALO), :] = jnp.zeros((HALO, D), f32)
            layernorm_to(0)

        def phase_a(first):
            j = step - 1
            base = pl.multiple_of(j * M, M)
            xn = xn_s[pl.ds(base, M), :]
            layernorm_to(pl.multiple_of(jnp.minimum(j + 1, NT - 1) * M, M))
            for part, dst in enumerate((q_s, k_s, v_s)):
                if first:
                    cp_qkv(part).wait()
                y = jnp.dot(xn, wqkv_v[:, part * D:(part + 1) * D], preferred_element_type=f32)
                if part == 0:
                    y = y * scale
                t = twist([y[:, c * 128:(c + 1) * 128] for c in range(8)])
                off = base + (HALO if part else 0)
                for m in range(8):
                    dst[pl.ds(off, M), m * 128:(m + 1) * 128] = t[m]

        if peel:
            @pl.when(step == 1)
            def _():
                phase_a(True)

            @pl.when(jnp.logical_and(step > 1, step <= NT))
            def _():
                phase_a(False)
        else:
            @pl.when(step == 1)
            def _():
                for p in range(3):
                    cp_qkv(p).wait()

            @pl.when(jnp.logical_and(step >= 1, step <= NT))
            def _():
                phase_a(False)

        @pl.when(step == NT + 1)
        def _():
            for i in range(4):
                cp_rest(i).wait()

        def attention(base, r0):
            def shifted(ref, m):
                kk = ref[pl.ds(base + r0, R + HALO), m * 128:(m + 1) * 128]
                out = [None] * W
                for r in range(4):
                    a = kk[8 - 2 * r: 8 - 2 * r + R + 8]
                    out[r] = a[8:R + 8]
                    out[r + 4] = a[0:R]
                return out
            prods = [[] for _ in range(W)]
            for m in range(8):
                qm = q_s[pl.ds(base + r0, R), m * 128:(m + 1) * 128]
                ks = shifted(k_s, m)
                for w in range(W):
                    prods[w].append(qm * ks[w])
            lane = lax.broadcasted_iota(jnp.int32, (R, 128), 1)
            pos = base + r0 + lax.broadcasted_iota(jnp.int32, (R, 128), 0)
            logits = []
            for w in range(W):
                l = _tree_sum(prods[w])
                l = l + jnp.take_along_axis(l, lane ^ 1, axis=1)
                l = l + jnp.take_along_axis(l, lane ^ 2, axis=1)
                if w > 0:
                    l = jnp.where(pos >= DIL * w, l, -1e9)
                logits.append(l)
            mx = functools.reduce(jnp.maximum, logits)
            es = [jnp.exp(l - mx) for l in logits]
            den = _tree_sum(es)
            inv = 1.0 / den
            a = [e * inv for e in es]
            ot = []
            for m in range(8):
                vs = shifted(v_s, m)
                ot.append(_tree_sum([a[w] * vs[w] for w in range(W)]))
            o = untwist(ot)
            o_s[pl.ds(r0, R), :] = jnp.concatenate(o, axis=1).astype(bf16)

        @pl.when(step > NT)
        def _():
            i = step - (NT + 1)
            base = pl.multiple_of(i * M, M)
            xn = xn_s[pl.ds(base, M), :]
            nsub = M // R
            done = 0
            if order == "first":
                for t in range(nsub):
                    attention(base, t * R)
                done = nsub
            acc = None
            for c in range(NC):
                g = jnp.dot(xn, wg_v[:, c * FC:(c + 1) * FC], preferred_element_type=f32)
                u = jnp.dot(xn, wu_v[:, c * FC:(c + 1) * FC], preferred_element_type=f32)
                h = (silu(g) * u).astype(bf16)
                d = jnp.dot(h, wd_v[c * FC:(c + 1) * FC, :], preferred_element_type=f32)
                acc = d if acc is None else acc + d
                tgt = min(nsub, ((c + 1) * nsub + NC - 2) // max(NC - 1, 1))
                while done < tgt:
                    attention(base, done * R)
                    done += 1
            while done < nsub:
                attention(base, done * R)
                done += 1
            gate = silu(acc)
            s = jnp.dot(o_s[...], wo_v[...], preferred_element_type=f32)
            out_ref[...] = (x_ref[...].astype(f32) + s * gate).astype(out_ref.dtype)

    def fn(A_x, A_wqkv, A_wo, B_x, B_w_gate, B_w_up, B_w_down):
        x2 = A_x.reshape(S, D)
        anyspec = pl.BlockSpec(memory_space=pl.ANY)
        def x_map(s):
            return (jnp.where(s <= NT, jnp.minimum(s, NT - 1), s - (NT + 1)), 0)
        out = pl.pallas_call(
            kernel,
            grid=(2 * NT + 1,),
            in_specs=[pl.BlockSpec((M, D), x_map), anyspec, anyspec, anyspec, anyspec, anyspec],
            out_specs=pl.BlockSpec((M, D), lambda s: (jnp.maximum(s - (NT + 1), 0), 0)),
            out_shape=jax.ShapeDtypeStruct((S, D), bf16),
            scratch_shapes=[
                pltpu.VMEM((D, 3 * D), bf16), pltpu.VMEM((D, D), bf16),
                pltpu.VMEM((D, F), bf16), pltpu.VMEM((D, F), bf16), pltpu.VMEM((F, D), bf16),
                pltpu.VMEM((S, D), bf16), pltpu.VMEM((S, D), f32),
                pltpu.VMEM((S + HALO, D), f32), pltpu.VMEM((S + HALO, D), f32),
                pltpu.VMEM((M, D), bf16),
                pltpu.SemaphoreType.DMA((7,)),
            ],
            compiler_params=pltpu.CompilerParams(
                dimension_semantics=("arbitrary",), vmem_limit_bytes=vmem_mb * 1024 * 1024),
        )(x2, A_wqkv, A_wo, B_w_gate, B_w_up, B_w_down)
        return out.reshape(1, S, D)
    return fn

pallas_recurrent_scan__sliding_local_dilated__swiglu_ffn__prompt_kernel = jax.jit(make(peel=False))
```

```python
import functools, os, contextlib
import jax
import jax.numpy as jnp
import numpy as np
from jax import lax
import jax.experimental.pallas as pl
import jax.experimental.pallas.tpu as pltpu

S, D, F, H, DH = 2048, 1024, 3584, 32, 32
W, DIL = 8, 2
HALO = 16
HD, HF = D // 2, F // 2
f32, bf16, i32 = jnp.float32, jnp.bfloat16, jnp.int32
scope = (lambda n: jax.named_scope(n)) if os.environ.get('SCOPES') else (lambda n: contextlib.nullcontext())
EVEN = {'XLA_TPU_EVENLY_DISTRIBUTE_CRITICAL_NODES': True}


def _level(a, b, bit, lane):
    lo = (lane & (1 << bit)) == 0
    x = jnp.where(lo, a, b)
    y = jnp.take_along_axis(jnp.where(lo, b, a), lane ^ (1 << bit), axis=1)
    return x, y


def _unlevel(x, y, bit, lane):
    lo = (lane & (1 << bit)) == 0
    yp = jnp.take_along_axis(y, lane ^ (1 << bit), axis=1)
    return jnp.where(lo, x, yp), jnp.where(lo, yp, x)


def twist(c):
    lane = lax.broadcasted_iota(i32, c[0].shape, 1)
    n = [None] * 8
    for p in range(4):
        n[p], n[4 + p] = _level(c[2 * p], c[2 * p + 1], 4, lane)
    c, n = n, [None] * 8
    for g in range(2):
        for p in range(2):
            n[g * 4 + p], n[g * 4 + 2 + p] = _level(c[g * 4 + 2 * p], c[g * 4 + 2 * p + 1], 3, lane)
    c, n = n, [None] * 8
    for g in range(4):
        n[g * 2], n[g * 2 + 1] = _level(c[g * 2], c[g * 2 + 1], 2, lane)
    return n


def untwist(t):
    lane = lax.broadcasted_iota(i32, t[0].shape, 1)
    n = [None] * 8
    for g in range(4):
        n[g * 2], n[g * 2 + 1] = _unlevel(t[g * 2], t[g * 2 + 1], 2, lane)
    c, n = n, [None] * 8
    for g in range(2):
        for p in range(2):
            n[g * 4 + 2 * p], n[g * 4 + 2 * p + 1] = _unlevel(c[g * 4 + p], c[g * 4 + 2 + p], 3, lane)
    c, n = n, [None] * 8
    for p in range(4):
        n[2 * p], n[2 * p + 1] = _unlevel(c[p], c[4 + p], 4, lane)
    return n


def _tree_sum(xs):
    xs = list(xs)
    while len(xs) > 1:
        nxt = [xs[i] + xs[i + 1] for i in range(0, len(xs) - 1, 2)]
        if len(xs) % 2:
            nxt.append(xs[-1])
        xs = nxt
    return xs[0]


def dot(a, b):
    return jnp.dot(a, b, preferred_element_type=f32)


def a_operands(a11, a12, a21, a22):
    return [(a11 + a22).astype(bf16), (a21 + a22).astype(bf16), a11.astype(bf16), a22.astype(bf16),
            (a11 + a12).astype(bf16), (a21 - a11).astype(bf16), (a12 - a22).astype(bf16)]


def combine(m):
    return (m[0] + m[3] - m[4] + m[6], m[2] + m[4], m[1] + m[3], m[0] - m[1] + m[2] + m[5])


def quarters(x):
    hm, hk = x.shape[0] // 2, x.shape[1] // 2
    return x[:hm, :hk], x[:hm, hk:], x[hm:, :hk], x[hm:, hk:]


def b_operand(raw, ext, i, hk, hn, k0, kn, n0, nn, c0=0):
    if i in (0, 5, 6):
        e = {0: 0, 5: 1, 6: 2}[i]
        return ext[e, k0:k0 + kn, c0 // 2 + n0:c0 // 2 + n0 + nn]
    r, c = {1: (0, 0), 2: (0, 1), 3: (1, 0), 4: (1, 1)}[i]
    return raw[r * hk + k0:r * hk + k0 + kn, c0 + c * hn + n0:c0 + c * hn + n0 + nn]


def make(M=256, CN=256, R=32, silu_mode="tanh", vmem_mb=120, TRT=128, TRS=64, flags=EVEN, qdt=f32):
    NT = S // M
    HM = M // 2
    NC = HF // CN
    NSUB = M // R
    exp_c = float(DH ** -0.5 * np.log2(np.e))

    def silu(g):
        if silu_mode == "sig":
            return g * jax.nn.sigmoid(g)
        hg = 0.5 * g
        return hg * jnp.tanh(hg) + hg

    def kernel(x_h, wqkv_h, wo_h, wg_h, wu_h, wd_h, out_ref,
               x_s, wqkv_v, wo_v, wg_v, wu_v, wd_v, wqkv_e, wo_e, wg_e, wu_e, wd_e,
               xa_s, q_s, k_s, v_s, o_s, sems):
        step = pl.program_id(0)

        def cp_x(t):
            sl = pl.ds(t * M, M) if t < 2 else pl.ds(2 * M, S - 2 * M)
            return pltpu.make_async_copy(x_h.at[sl, :], x_s.at[sl, :], sems.at[7 + t])
        def cp_qkv(p):
            return pltpu.make_async_copy(wqkv_h.at[:, pl.ds(p * D, D)], wqkv_v.at[:, pl.ds(p * D, D)], sems.at[p])
        rest = [(wg_h, wg_v), (wu_h, wu_v), (wd_h, wd_v), (wo_h, wo_v)]
        def cp_rest(i):
            return pltpu.make_async_copy(rest[i][0], rest[i][1], sems.at[3 + i])

        def layernorm(t):
            x = x_s[pl.ds(pl.multiple_of(t * M, M), M), :].astype(f32)
            mu = jnp.mean(x, axis=-1, keepdims=True)
            xc = x - mu
            var = jnp.mean(xc * xc, axis=-1, keepdims=True)
            a = a_operands(*quarters(xc * lax.rsqrt(var + 1e-5)))
            for i in range(7):
                xa_s[i, pl.ds(pl.multiple_of(t * HM, HM), HM), :] = a[i]

        def store_sums(raw, ext, top, bot, hk, hn, c0, blocks):
            b11, b12, b21, b22 = [b.astype(f32) for b in blocks]
            ext[0, top, pl.ds(c0 // 2, hn)] = (b11 + b22).astype(bf16)
            ext[1, top, pl.ds(c0 // 2, hn)] = (b11 + b12).astype(bf16)
            ext[2, top, pl.ds(c0 // 2, hn)] = (b21 + b22).astype(bf16)
            raw[top, pl.ds(c0 + hn, hn)] = (b12 - b22).astype(bf16)
            raw[bot, pl.ds(c0, hn)] = (b21 - b11).astype(bf16)

        def prep_plain(raw, ext, hk, hn, tr):
            def body(r, carry):
                top = pl.ds(pl.multiple_of(r * tr, tr), tr)
                bot = pl.ds(pl.multiple_of(hk + r * tr, tr), tr)
                store_sums(raw, ext, top, bot, hk, hn, 0,
                           (raw[top, 0:hn], raw[top, hn:2 * hn], raw[bot, 0:hn], raw[bot, hn:2 * hn]))
                return carry
            lax.fori_loop(0, hk // tr, body, 0)

        def prep_qkv(p):
            def body(r, carry):
                top = pl.ds(pl.multiple_of(r * TRT, TRT), TRT)
                bot = pl.ds(pl.multiple_of(HD + r * TRT, TRT), TRT)
                tw = []
                for rows in (top, bot):
                    w = pltpu.bitcast(wqkv_v[rows, pl.ds(p * D, D)], i32)
                    t = twist([w[:, c * 128:(c + 1) * 128] for c in range(8)])
                    tw.append(pltpu.bitcast(jnp.concatenate(t[:4], axis=1), bf16))
                    tw.append(pltpu.bitcast(jnp.concatenate(t[4:], axis=1), bf16))
                wqkv_v[top, pl.ds(p * D, HD)] = tw[0]
                wqkv_v[bot, pl.ds(p * D + HD, HD)] = tw[3]
                store_sums(wqkv_v, wqkv_e, top, bot, HD, HD, p * D, tw)
                return carry
            lax.fori_loop(0, HD // TRT, body, 0)

        def prologue():
            cp_qkv(0).start()
            cp_x(0).start()
            cp_x(1).start()
            cp_qkv(1).start()
            cp_qkv(2).start()
            cp_x(2).start()
            for i in range(4):
                cp_rest(i).start()
            k_s[pl.ds(0, HALO), :] = jnp.zeros((HALO, D), f32)
            v_s[pl.ds(0, HALO), :] = jnp.zeros((HALO, D), f32)
            cp_qkv(0).wait()
            prep_qkv(0)
            cp_x(0).wait()
            layernorm(0)
            cp_x(1).wait()
        with scope('pro'):
            pl.when(step == 0)(prologue)

        def phase_a():
            j = step - 1
            rows = pl.ds(pl.multiple_of(j * HM, HM), HM)
            base = pl.multiple_of(j * M, M)
            a = [xa_s[i, rows, :] for i in range(7)]

            @pl.when(step == 2)
            def _():
                cp_x(2).wait()
            for part, dst in enumerate((q_s, k_s, v_s)):
                if part > 0:
                    @pl.when(step == 1)
                    def _():
                        cp_qkv(part).wait()
                        prep_qkv(part)
                c = combine([dot(a[i], b_operand(wqkv_v, wqkv_e, i, HD, HD, 0, HD, 0, HD, part * D)) for i in range(7)])
                off = base + (HALO if part else 0)
                for bi, blk in enumerate(c):
                    dst[pl.ds(off + (bi // 2) * HM, HM), (bi % 2) * HD:(bi % 2 + 1) * HD] = blk.astype(dst.dtype)
                if part == 0:
                    layernorm(jnp.minimum(j + 1, NT - 1))
        with scope('A'):
            pl.when(jnp.logical_and(step >= 1, step <= NT))(phase_a)

        def prep_rest():
            for i in range(4):
                cp_rest(i).wait()
            prep_plain(wg_v, wg_e, HD, HF, TRS)
            prep_plain(wu_v, wu_e, HD, HF, TRS)
            prep_plain(wd_v, wd_e, HF, HD, 224)
            prep_plain(wo_v, wo_e, HD, HD, 128)
        with scope('prepB'):
            pl.when(step == NT + 1)(prep_rest)

        def attention(base, r0):
            def shifted(ref, m):
                kk = ref[pl.ds(base + r0, R + HALO), m * 128:(m + 1) * 128]
                out = [None] * W
                for r in range(4):
                    a = kk[8 - 2 * r: 8 - 2 * r + R + 8]
                    out[r] = a[8:R + 8]
                    out[r + 4] = a[0:R]
                return out
            prods = [[] for _ in range(W)]
            for m in range(8):
                qm = q_s[pl.ds(base + r0, R), m * 128:(m + 1) * 128].astype(f32)
                ks = shifted(k_s, m)
                for w in range(W):
                    prods[w].append(qm * ks[w])
            lane = lax.broadcasted_iota(i32, (R, 128), 1)
            pos = base + r0 + lax.broadcasted_iota(i32, (R, 128), 0)
            logits = []
            for w in range(W):
                l = _tree_sum(prods[w])
                l = l + jnp.take_along_axis(l, lane ^ 1, axis=1)
                l = l + jnp.take_along_axis(l, lane ^ 2, axis=1)
                if w > 0:
                    l = jnp.where(pos >= DIL * w, l, -1e9)
                logits.append(l)
            mx = functools.reduce(jnp.maximum, logits)
            es = [jnp.exp2((l - mx) * exp_c) for l in logits]
            inv = 1.0 / _tree_sum(es)
            a = [e * inv for e in es]
            ot = []
            for m in range(8):
                vs = shifted(v_s, m)
                ot.append(_tree_sum([a[w] * vs[w] for w in range(W)]))
            o_s[pl.ds(r0, R), :] = jnp.concatenate(untwist(ot), axis=1)

        def phase_b():
            t = step - (NT + 1)
            base = pl.multiple_of(t * M, M)
            rows = pl.ds(pl.multiple_of(t * HM, HM), HM)
            a = [xa_s[i, rows, :] for i in range(7)]
            done = 0
            md = [None] * 7
            for c in range(NC):
                g = combine([dot(a[i], b_operand(wg_v, wg_e, i, HD, HF, 0, HD, c * CN, CN)) for i in range(7)])
                u = combine([dot(a[i], b_operand(wu_v, wu_e, i, HD, HF, 0, HD, c * CN, CN)) for i in range(7)])
                e = a_operands(*[silu(g[i]) * u[i] for i in range(4)])
                for i in range(7):
                    d = dot(e[i], b_operand(wd_v, wd_e, i, HF, HD, c * CN, CN, 0, HD))
                    md[i] = d if md[i] is None else md[i] + d
                tgt = min(NSUB, ((c + 1) * NSUB + NC - 1) // NC)
                while done < tgt:
                    attention(base, done * R); done += 1
            gate = [silu(y) for y in combine(md)]
            oa = a_operands(o_s[0:HM, 0:HD], o_s[0:HM, HD:D], o_s[HM:M, 0:HD], o_s[HM:M, HD:D])
            s = combine([dot(oa[i], b_operand(wo_v, wo_e, i, HD, HD, 0, HD, 0, HD)) for i in range(7)])
            for bi in range(4):
                r0, c0 = (bi // 2) * HM, (bi % 2) * HD
                xr = x_s[pl.ds(base + r0, HM), c0:c0 + HD].astype(f32)
                out_ref[r0:r0 + HM, c0:c0 + HD] = (xr + s[bi] * gate[bi]).astype(out_ref.dtype)
        with scope('B'):
            pl.when(step > NT)(phase_b)

    def fn(A_x, A_wqkv, A_wo, B_x, B_w_gate, B_w_up, B_w_down):
        x2 = A_x.reshape(S, D)
        anyspec = pl.BlockSpec(memory_space=pl.ANY)
        out = pl.pallas_call(
            kernel,
            grid=(2 * NT + 1,),
            in_specs=[anyspec] * 6,
            out_specs=pl.BlockSpec((M, D), lambda s: (jnp.maximum(s - (NT + 1), 0), 0)),
            out_shape=jax.ShapeDtypeStruct((S, D), bf16),
            scratch_shapes=[
                pltpu.VMEM((S, D), bf16),
                pltpu.VMEM((D, 3 * D), bf16), pltpu.VMEM((D, D), bf16),
                pltpu.VMEM((D, F), bf16), pltpu.VMEM((D, F), bf16), pltpu.VMEM((F, D), bf16),
                pltpu.VMEM((3, HD, 3 * HD), bf16), pltpu.VMEM((3, HD, HD), bf16),
                pltpu.VMEM((3, HD, HF), bf16), pltpu.VMEM((3, HD, HF), bf16), pltpu.VMEM((3, HF, HD), bf16),
                pltpu.VMEM((7, S // 2, HD), bf16), pltpu.VMEM((S, D), qdt),
                pltpu.VMEM((S + HALO, D), f32), pltpu.VMEM((S + HALO, D), f32),
                pltpu.VMEM((M, D), f32),
                pltpu.SemaphoreType.DMA((10,)),
            ],
            compiler_params=pltpu.CompilerParams(
                dimension_semantics=("arbitrary",), vmem_limit_bytes=vmem_mb * 1024 * 1024, flags=flags),
        )(x2, A_wqkv, A_wo, B_w_gate, B_w_up, B_w_down)
        return out.reshape(1, S, D)
    return fn

pallas_recurrent_scan__sliding_local_dilated__swiglu_ffn__prompt_kernel = jax.jit(make(CN=896))
```

```python
import functools, os, contextlib
import jax
import jax.numpy as jnp
import numpy as np
from jax import lax
import jax.experimental.pallas as pl
import jax.experimental.pallas.tpu as pltpu

S, D, F, H, DH = 2048, 1024, 3584, 32, 32
W, DIL = 8, 2
HALO = 16
HD, HF = D // 2, F // 2
f32, bf16, i32 = jnp.float32, jnp.bfloat16, jnp.int32
scope = (lambda n: jax.named_scope(n)) if os.environ.get('SCOPES') else (lambda n: contextlib.nullcontext())
EVEN = {'XLA_TPU_EVENLY_DISTRIBUTE_CRITICAL_NODES': True}


def _level(a, b, bit, lane):
    lo = (lane & (1 << bit)) == 0
    x = jnp.where(lo, a, b)
    y = jnp.take_along_axis(jnp.where(lo, b, a), lane ^ (1 << bit), axis=1)
    return x, y


def _unlevel(x, y, bit, lane):
    lo = (lane & (1 << bit)) == 0
    yp = jnp.take_along_axis(y, lane ^ (1 << bit), axis=1)
    return jnp.where(lo, x, yp), jnp.where(lo, yp, x)


def twist(c):
    lane = lax.broadcasted_iota(i32, c[0].shape, 1)
    n = [None] * 8
    for p in range(4):
        n[p], n[4 + p] = _level(c[2 * p], c[2 * p + 1], 4, lane)
    c, n = n, [None] * 8
    for g in range(2):
        for p in range(2):
            n[g * 4 + p], n[g * 4 + 2 + p] = _level(c[g * 4 + 2 * p], c[g * 4 + 2 * p + 1], 3, lane)
    c, n = n, [None] * 8
    for g in range(4):
        n[g * 2], n[g * 2 + 1] = _level(c[g * 2], c[g * 2 + 1], 2, lane)
    return n


def untwist(t):
    lane = lax.broadcasted_iota(i32, t[0].shape, 1)
    n = [None] * 8
    for g in range(4):
        n[g * 2], n[g * 2 + 1] = _unlevel(t[g * 2], t[g * 2 + 1], 2, lane)
    c, n = n, [None] * 8
    for g in range(2):
        for p in range(2):
            n[g * 4 + 2 * p], n[g * 4 + 2 * p + 1] = _unlevel(c[g * 4 + p], c[g * 4 + 2 + p], 3, lane)
    c, n = n, [None] * 8
    for p in range(4):
        n[2 * p], n[2 * p + 1] = _unlevel(c[p], c[4 + p], 4, lane)
    return n


def _tree_sum(xs):
    xs = list(xs)
    while len(xs) > 1:
        nxt = [xs[i] + xs[i + 1] for i in range(0, len(xs) - 1, 2)]
        if len(xs) % 2:
            nxt.append(xs[-1])
        xs = nxt
    return xs[0]


def dot(a, b):
    return jnp.dot(a, b, preferred_element_type=f32)


def a_operands(a11, a12, a21, a22):
    return [(a11 + a22).astype(bf16), (a21 + a22).astype(bf16), a11.astype(bf16), a22.astype(bf16),
            (a11 + a12).astype(bf16), (a21 - a11).astype(bf16), (a12 - a22).astype(bf16)]


def combine(m):
    return (m[0] + m[3] - m[4] + m[6], m[2] + m[4], m[1] + m[3], m[0] - m[1] + m[2] + m[5])


def quarters(x):
    hm, hk = x.shape[0] // 2, x.shape[1] // 2
    return x[:hm, :hk], x[:hm, hk:], x[hm:, :hk], x[hm:, hk:]


def b_operand(raw, ext, i, hn, k0, kn, n0, nn, c0=0):
    if i in (1, 4):
        r = 0 if i == 1 else 1
        return raw[r, k0:k0 + kn, c0 + r * hn + n0:c0 + r * hn + n0 + nn]
    e = {0: 0, 2: 1, 3: 2, 5: 3, 6: 4}[i]
    return ext[e, k0:k0 + kn, c0 // 2 + n0:c0 // 2 + n0 + nn]


def make(M=256, CN=896, R=32, silu_mode="tanh", vmem_mb=120, TRT=128, TRS=64, flags=EVEN, qdt=f32, prep_after=2, RB=16, CB=256, hoist=False, noprep=False, anchor=True, ln_after=0):
    NT = S // M
    HM = M // 2
    NC = HF // CN
    NSUB = M // R
    exp_c = float(DH ** -0.5 * np.log2(np.e))

    def silu(g):
        if silu_mode == "sig":
            return g * jax.nn.sigmoid(g)
        hg = 0.5 * g
        return hg * jnp.tanh(hg) + hg

    def kernel(x_h, wqkv_h, wo_h, wg_h, wu_h, wd_h, out_ref,
               x_s, wqkv_v, wo_v, wg_v, wu_v, wd_v, wqkv_e, wo_e, wg_e, wu_e, wd_e,
               xa_s, q_s, k_s, v_s, o_s, sems):
        step = pl.program_id(0)
        zero = jnp.minimum(step, 0)

        def cp_x(t):
            sl = pl.ds(t * M, M) if t < 2 else pl.ds(2 * M, S - 2 * M)
            return pltpu.make_async_copy(x_h.at[sl, :], x_s.at[sl, :], sems.at[3 + t])
        def cp_qkv(p):
            return pltpu.make_async_copy(wqkv_h.at[:, :, pl.ds(p * D, D)], wqkv_v.at[:, :, pl.ds(p * D, D)], sems.at[p])
        rest = [(wg_h, wg_v, HD // NT), (wu_h, wu_v, HD // NT), (wd_h, wd_v, HF // NT), (wo_h, wo_v, HD // NT)]
        def cp_rest(j):
            out = []
            for src, dst, n in rest:
                sl = pl.ds(pl.multiple_of(j * n, n), n)
                out.append(pltpu.make_async_copy(src.at[:, sl, :], dst.at[:, sl, :], sems.at[6 + j]))
            return out

        def layernorm(t):
            x = x_s[pl.ds(pl.multiple_of(t * M, M), M), :].astype(f32)
            mu = jnp.mean(x, axis=-1, keepdims=True)
            xc = x - mu
            var = jnp.mean(xc * xc, axis=-1, keepdims=True)
            a = a_operands(*quarters(xc * lax.rsqrt(var + 1e-5)))
            for i in range(7):
                xa_s[i, pl.ds(pl.multiple_of(t * (HM // 2), HM // 2), HM // 2), :] = pltpu.bitcast(a[i], i32)

        def load_a(i, t):
            return pltpu.bitcast(xa_s[i, pl.ds(pl.multiple_of(t * (HM // 2), HM // 2), HM // 2), :], bf16)

        def store_sums(ext, rows, cols, b11, b12, b21, b22):
            b11, b12, b21, b22 = [b.astype(f32) for b in (b11, b12, b21, b22)]
            ext[0, rows, cols] = (b11 + b22).astype(bf16)
            ext[1, rows, cols] = (b12 - b22).astype(bf16)
            ext[2, rows, cols] = (b21 - b11).astype(bf16)
            ext[3, rows, cols] = (b11 + b12).astype(bf16)
            ext[4, rows, cols] = (b21 + b22).astype(bf16)

        def prep_plain(raw, ext, r0, n, hn, rb, cb):
            for r in range(0, n, rb):
                rows = pl.ds(pl.multiple_of(r0 + r, rb), rb)
                for c in range(0, hn, cb):
                    b11, b22 = raw[0, rows, c:c + cb], raw[1, rows, hn + c:hn + c + cb]
                    if anchor:
                        b11, b22 = [jnp.concatenate([pltpu.bitcast(pltpu.roll(pltpu.bitcast(b[:, k:k + 128], i32), zero, 1), bf16)
                                                     for k in range(0, cb, 128)], axis=1) for b in (b11, b22)]
                    store_sums(ext, rows, pl.ds(c, cb), b11, raw[0, rows, hn + c:hn + c + cb], raw[1, rows, c:c + cb], b22)

        def prep_qkv(p):
            def body(r, carry):
                rows = pl.ds(pl.multiple_of(r * TRT, TRT), TRT)
                tw = []
                for half in range(2):
                    w = pltpu.bitcast(wqkv_v[half, rows, pl.ds(p * D, D)], i32)
                    t = twist([w[:, c * 128:(c + 1) * 128] for c in range(8)])
                    tw.append(pltpu.bitcast(jnp.concatenate(t[:4], axis=1), bf16))
                    tw.append(pltpu.bitcast(jnp.concatenate(t[4:], axis=1), bf16))
                wqkv_v[0, rows, pl.ds(p * D, HD)] = tw[0]
                wqkv_v[1, rows, pl.ds(p * D + HD, HD)] = tw[3]
                store_sums(wqkv_e, rows, pl.ds(p * HD, HD), *tw)
                return carry
            lax.fori_loop(0, HD // TRT, body, 0)

        def prologue():
            cp_qkv(0).start()
            cp_x(0).start()
            cp_qkv(1).start()
            cp_x(1).start()
            cp_qkv(2).start()
            for c in cp_rest(0):
                c.start()
            cp_x(2).start()
            def start_chunk(j, carry):
                for c in cp_rest(j):
                    c.start()
                return carry
            lax.fori_loop(1, NT, start_chunk, 0)
            k_s[pl.ds(0, HALO), :] = jnp.zeros((HALO, D), f32)
            v_s[pl.ds(0, HALO), :] = jnp.zeros((HALO, D), f32)
            cp_qkv(0).wait()
            prep_qkv(0)
            cp_x(0).wait()
            layernorm(0)
            cp_qkv(1).wait()
            prep_qkv(1)
            cp_x(1).wait()
            cp_qkv(2).wait()
            prep_qkv(2)
        with scope('pro'):
            pl.when(step == 0)(prologue)

        def phase_a():
            j = step - 1
            base = pl.multiple_of(j * M, M)
            if not hoist:
                @pl.when(step == 2)
                def _():
                    cp_x(2).wait()
                for c in cp_rest(j):
                    c.wait()
            js = (j, jnp.minimum(j, NT - 1), jnp.maximum(j, 0))
            for part, dst in enumerate((q_s, k_s, v_s)):
                c = combine([dot(load_a(i, js[part]), b_operand(wqkv_v, wqkv_e, i, HD, 0, HD, 0, HD, part * D)) for i in range(7)])
                off = base + (HALO if part else 0)
                for bi, blk in enumerate(c):
                    dst[pl.ds(off + (bi // 2) * HM, HM), (bi % 2) * HD:(bi % 2 + 1) * HD] = blk.astype(dst.dtype)
                if part == ln_after:
                    layernorm(jnp.minimum(j + 1, NT - 1))
                if part == prep_after and not noprep:
                    for (src, raw, n), ext, hn in zip(rest, (wg_e, wu_e, wd_e, wo_e), (HF, HF, HD, HD)):
                        prep_plain(raw, ext, j * n, n, hn, RB, CB)
        if hoist:
            @pl.when(jnp.logical_and(step >= 1, step <= NT))
            def _():
                @pl.when(step == 2)
                def _():
                    cp_x(2).wait()
                for c in cp_rest(step - 1):
                    c.wait()
        with scope('A'):
            pl.when(jnp.logical_and(step >= 1, step <= NT))(phase_a)

        def attention(base, r0):
            def shifted(ref, m):
                kk = ref[pl.ds(base + r0, R + HALO), m * 128:(m + 1) * 128]
                out = [None] * W
                for r in range(4):
                    a = kk[8 - 2 * r: 8 - 2 * r + R + 8]
                    out[r] = a[8:R + 8]
                    out[r + 4] = a[0:R]
                return out
            prods = [[] for _ in range(W)]
            for m in range(8):
                qm = q_s[pl.ds(base + r0, R), m * 128:(m + 1) * 128].astype(f32)
                ks = shifted(k_s, m)
                for w in range(W):
                    prods[w].append(qm * ks[w])
            lane = lax.broadcasted_iota(i32, (R, 128), 1)
            pos = base + r0 + lax.broadcasted_iota(i32, (R, 128), 0)
            logits = []
            for w in range(W):
                l = _tree_sum(prods[w])
                l = l + jnp.take_along_axis(l, lane ^ 1, axis=1)
                l = l + jnp.take_along_axis(l, lane ^ 2, axis=1)
                if w > 0:
                    l = jnp.where(pos >= DIL * w, l, -1e9)
                logits.append(l)
            mx = functools.reduce(jnp.maximum, logits)
            es = [jnp.exp2((l - mx) * exp_c) for l in logits]
            inv = 1.0 / _tree_sum(es)
            a = [e * inv for e in es]
            ot = []
            for m in range(8):
                vs = shifted(v_s, m)
                ot.append(_tree_sum([a[w] * vs[w] for w in range(W)]))
            o_s[pl.ds(r0, R), :] = jnp.concatenate(untwist(ot), axis=1)

        def phase_b():
            t = step - (NT + 1)
            base = pl.multiple_of(t * M, M)
            ts = (t, jnp.minimum(t, NT - 1), jnp.maximum(t, 0), jnp.clip(t, 0, NT))
            done = 0
            md = [None] * 7
            for c in range(NC):
                g = combine([dot(load_a(i, ts[(2 * c) % 4]), b_operand(wg_v, wg_e, i, HF, 0, HD, c * CN, CN)) for i in range(7)])
                u = combine([dot(load_a(i, ts[(2 * c + 1) % 4]), b_operand(wu_v, wu_e, i, HF, 0, HD, c * CN, CN)) for i in range(7)])
                e = a_operands(*[silu(g[i]) * u[i] for i in range(4)])
                for i in range(7):
                    d = dot(e[i], b_operand(wd_v, wd_e, i, HD, c * CN, CN, 0, HD))
                    md[i] = d if md[i] is None else md[i] + d
                tgt = min(NSUB, ((c + 1) * NSUB + NC - 1) // NC)
                while done < tgt:
                    attention(base, done * R); done += 1
            gate = [silu(y) for y in combine(md)]
            oa = a_operands(o_s[0:HM, 0:HD], o_s[0:HM, HD:D], o_s[HM:M, 0:HD], o_s[HM:M, HD:D])
            s = combine([dot(oa[i], b_operand(wo_v, wo_e, i, HD, 0, HD, 0, HD)) for i in range(7)])
            for bi in range(4):
                r0, c0 = (bi // 2) * HM, (bi % 2) * HD
                xr = x_s[pl.ds(base + r0, HM), c0:c0 + HD].astype(f32)
                out_ref[r0:r0 + HM, c0:c0 + HD] = (xr + s[bi] * gate[bi]).astype(out_ref.dtype)
        with scope('B'):
            pl.when(step > NT)(phase_b)

    def fn(A_x, A_wqkv, A_wo, B_x, B_w_gate, B_w_up, B_w_down):
        x2 = A_x.reshape(S, D)
        anyspec = pl.BlockSpec(memory_space=pl.ANY)
        out = pl.pallas_call(
            kernel,
            grid=(2 * NT + 1,),
            in_specs=[anyspec] * 6,
            out_specs=pl.BlockSpec((M, D), lambda s: (jnp.maximum(s - (NT + 1), 0), 0)),
            out_shape=jax.ShapeDtypeStruct((S, D), bf16),
            scratch_shapes=[
                pltpu.VMEM((S, D), bf16),
                pltpu.VMEM((2, HD, 3 * D), bf16), pltpu.VMEM((2, HD, D), bf16),
                pltpu.VMEM((2, HD, F), bf16), pltpu.VMEM((2, HD, F), bf16), pltpu.VMEM((2, HF, D), bf16),
                pltpu.VMEM((5, HD, 3 * HD), bf16), pltpu.VMEM((5, HD, HD), bf16),
                pltpu.VMEM((5, HD, HF), bf16), pltpu.VMEM((5, HD, HF), bf16), pltpu.VMEM((5, HF, HD), bf16),
                pltpu.VMEM((7, S // 4, HD), i32), pltpu.VMEM((S, D), qdt),
                pltpu.VMEM((S + HALO, D), f32), pltpu.VMEM((S + HALO, D), f32),
                pltpu.VMEM((M, D), f32),
                pltpu.SemaphoreType.DMA((6 + NT,)),
            ],
            compiler_params=pltpu.CompilerParams(
                dimension_semantics=("arbitrary",), vmem_limit_bytes=vmem_mb * 1024 * 1024, flags=flags),
        )(x2, A_wqkv.reshape(2, HD, 3 * D), A_wo.reshape(2, HD, D), B_w_gate.reshape(2, HD, F),
          B_w_up.reshape(2, HD, F), B_w_down.reshape(2, HF, D))
        return out.reshape(1, S, D)
    return fn

pallas_recurrent_scan__sliding_local_dilated__swiglu_ffn__prompt_kernel = jax.jit(make(ln_after=2))
```

```python
import functools, os, contextlib
import jax
import jax.numpy as jnp
import numpy as np
from jax import lax
import jax.experimental.pallas as pl
import jax.experimental.pallas.tpu as pltpu

S, D, F, H, DH = 2048, 1024, 3584, 32, 32
W, DIL = 8, 2
HALO = 16
HD, HF = D // 2, F // 2
f32, bf16, i32 = jnp.float32, jnp.bfloat16, jnp.int32
scope = (lambda n: jax.named_scope(n)) if os.environ.get('SCOPES') else (lambda n: contextlib.nullcontext())
EVEN = {'XLA_TPU_EVENLY_DISTRIBUTE_CRITICAL_NODES': True}


def _level(a, b, bit, lane):
    lo = (lane & (1 << bit)) == 0
    x = jnp.where(lo, a, b)
    y = jnp.take_along_axis(jnp.where(lo, b, a), lane ^ (1 << bit), axis=1)
    return x, y


def _unlevel(x, y, bit, lane):
    lo = (lane & (1 << bit)) == 0
    yp = jnp.take_along_axis(y, lane ^ (1 << bit), axis=1)
    return jnp.where(lo, x, yp), jnp.where(lo, yp, x)


def twist(c):
    lane = lax.broadcasted_iota(i32, c[0].shape, 1)
    n = [None] * 8
    for p in range(4):
        n[p], n[4 + p] = _level(c[2 * p], c[2 * p + 1], 4, lane)
    c, n = n, [None] * 8
    for g in range(2):
        for p in range(2):
            n[g * 4 + p], n[g * 4 + 2 + p] = _level(c[g * 4 + 2 * p], c[g * 4 + 2 * p + 1], 3, lane)
    c, n = n, [None] * 8
    for g in range(4):
        n[g * 2], n[g * 2 + 1] = _level(c[g * 2], c[g * 2 + 1], 2, lane)
    return n


def untwist(t):
    lane = lax.broadcasted_iota(i32, t[0].shape, 1)
    n = [None] * 8
    for g in range(4):
        n[g * 2], n[g * 2 + 1] = _unlevel(t[g * 2], t[g * 2 + 1], 2, lane)
    c, n = n, [None] * 8
    for g in range(2):
        for p in range(2):
            n[g * 4 + 2 * p], n[g * 4 + 2 * p + 1] = _unlevel(c[g * 4 + p], c[g * 4 + 2 + p], 3, lane)
    c, n = n, [None] * 8
    for p in range(4):
        n[2 * p], n[2 * p + 1] = _unlevel(c[p], c[4 + p], 4, lane)
    return n


def _tree_sum(xs):
    xs = list(xs)
    while len(xs) > 1:
        nxt = [xs[i] + xs[i + 1] for i in range(0, len(xs) - 1, 2)]
        if len(xs) % 2:
            nxt.append(xs[-1])
        xs = nxt
    return xs[0]


def dot(a, b):
    return jnp.dot(a, b, preferred_element_type=f32)


def a_operands(a11, a12, a21, a22):
    return [(a11 + a22).astype(bf16), (a21 + a22).astype(bf16), a11.astype(bf16), a22.astype(bf16),
            (a11 + a12).astype(bf16), (a21 - a11).astype(bf16), (a12 - a22).astype(bf16)]


def combine(m):
    return (m[0] + m[3] - m[4] + m[6], m[2] + m[4], m[1] + m[3], m[0] - m[1] + m[2] + m[5])


def quarters(x):
    hm, hk = x.shape[0] // 2, x.shape[1] // 2
    return x[:hm, :hk], x[:hm, hk:], x[hm:, :hk], x[hm:, hk:]


def b_operand(raw, ext, i, hn, k0, kn, n0, nn):
    if i in (1, 4):
        r = 0 if i == 1 else 1
        return raw[r, k0:k0 + kn, r * hn + n0:r * hn + n0 + nn]
    return ext[{0: 0, 2: 1, 3: 2, 5: 3, 6: 4}[i], k0:k0 + kn, n0:n0 + nn]


def b_sums(b11, b12, b21, b22):
    b11, b12, b21, b22 = [b.astype(f32) for b in (b11, b12, b21, b22)]
    return [(b11 + b22).astype(bf16), (b12 - b22).astype(bf16), (b21 - b11).astype(bf16),
            (b11 + b12).astype(bf16), (b21 + b22).astype(bf16)]


def make(M=256, CN=896, R=32, vmem_mb=120, flags=EVEN, RB=16, CB=256, QC=4, anchor=True, rest_early=False):
    NT = S // M
    HM = M // 2
    NC = HF // CN
    NSUB = M // R
    exp_c = float(DH ** -0.5 * np.log2(np.e))
    SX, SQ, SKV, SR = 0, NT, NT + QC, 2 * NT + QC

    def silu(g):
        hg = 0.5 * g
        return hg * jnp.tanh(hg) + hg

    def kernel(x_h, wqkv_h, wo_h, wg_h, wu_h, wd_h, out_ref,
               x_s, wqkv_v, wo_v, wg_v, wu_v, wd_v, opq, opk, opv, wo_e, wg_e, wu_e, wd_e,
               xa_s, q_s, k_s, v_s, o_s, sems):
        step = pl.program_id(0)
        zero = jnp.minimum(step, 0)

        def ds(i, n):
            return pl.ds(pl.multiple_of(i * n, n), n)

        def cp_x(t):
            return pltpu.make_async_copy(x_h.at[ds(t, M), :], x_s.at[ds(t, M), :], sems.at[SX + t])

        def cp_w(p, rows, sem):
            return pltpu.make_async_copy(wqkv_h.at[:, rows, pl.ds(p * D, D)], wqkv_v.at[:, rows, pl.ds(p * D, D)],
                                         sems.at[sem])

        def cp_q(r):
            return cp_w(0, ds(r, HD // QC), SQ + r)

        def cp_kv(j):
            return [cp_w(p, ds(j, HD // NT), SKV + j) for p in (1, 2)]

        rest = [(wg_h, wg_v, wg_e, HD // NT, HF), (wu_h, wu_v, wu_e, HD // NT, HF),
                (wd_h, wd_v, wd_e, HF // NT, HD), (wo_h, wo_v, wo_e, HD // NT, HD)]

        def cp_rest(j):
            return [pltpu.make_async_copy(src.at[:, ds(j, n), :], raw.at[:, ds(j, n), :], sems.at[SR + j])
                    for src, raw, _, n, _ in rest]

        def layernorm(t):
            x = x_s[ds(t, M), :].astype(f32)
            xc = x - jnp.mean(x, axis=-1, keepdims=True)
            var = jnp.mean(xc * xc, axis=-1, keepdims=True)
            a = a_operands(*quarters(xc * lax.rsqrt(var + 1e-5)))
            for i in range(7):
                xa_s[i, ds(t, HM // 2), :] = pltpu.bitcast(a[i], i32)

        def load_a(i, t):
            return pltpu.bitcast(xa_s[i, ds(t, HM // 2), :], bf16)

        def prep_part(p, op, rows):
            blk = []
            for half in range(2):
                w = pltpu.bitcast(wqkv_v[half, rows, pl.ds(p * D, D)], i32)
                t = twist([w[:, c * 128:(c + 1) * 128] for c in range(8)])
                blk += [pltpu.bitcast(jnp.concatenate(t[:4], axis=1), bf16),
                        pltpu.bitcast(jnp.concatenate(t[4:], axis=1), bf16)]
            e = b_sums(*blk)
            for i, v in zip((0, 2, 3, 5, 6, 1, 4), e + [blk[0], blk[3]]):
                op[i, rows, :] = v

        def prep_rest(j):
            for _, raw, ext, n, hn in rest:
                for r in range(0, n, RB):
                    rows = pl.ds(pl.multiple_of(j * n + r, RB), RB)
                    for c in range(0, hn, CB):
                        b11, b22 = raw[0, rows, c:c + CB], raw[1, rows, hn + c:hn + c + CB]
                        if anchor:
                            b11, b22 = [jnp.concatenate(
                                [pltpu.bitcast(pltpu.roll(pltpu.bitcast(b[:, k:k + 128], i32), zero, 1), bf16)
                                 for k in range(0, CB, 128)], axis=1) for b in (b11, b22)]
                        e = b_sums(b11, raw[0, rows, hn + c:hn + c + CB], raw[1, rows, c:c + CB], b22)
                        for i in range(5):
                            ext[i, rows, c:c + CB] = e[i]

        def qkv_dot(t, op, dst, off):
            c = combine([dot(load_a(i, t), op[i]) for i in range(7)])
            for bi, blk in enumerate(c):
                dst[pl.ds(pl.multiple_of(t * M, M) + off + (bi // 2) * HM, HM), (bi % 2) * HD:(bi % 2 + 1) * HD] = blk

        def prologue():
            cp_x(0).start()
            for r in range(QC):
                cp_q(r).start()

            def start_kv(j, carry):
                @pl.when(j < NT - 1)
                def _():
                    cp_x(j + 1).start()
                for c in cp_kv(j):
                    c.start()
                return carry
            lax.fori_loop(0, NT, start_kv, 0)
            if rest_early:
                def start_rest(j, carry):
                    for c in cp_rest(j):
                        c.start()
                    return carry
                lax.fori_loop(0, NT, start_rest, 0)
            k_s[pl.ds(0, HALO), :] = jnp.zeros((HALO, D), f32)
            v_s[pl.ds(0, HALO), :] = jnp.zeros((HALO, D), f32)
            cp_x(0).wait()
            layernorm(0)

            def prep_q(r, carry):
                cp_q(r).wait()
                prep_part(0, opq, ds(r, HD // QC))
                return carry
            lax.fori_loop(0, QC, prep_q, 0)

        def q_pass():
            j = step - 1
            if not rest_early:
                for c in cp_rest(j):
                    c.start()

            @pl.when(j < NT - 1)
            def _():
                cp_x(j + 1).wait()
            for c in cp_kv(j):
                c.wait()
            qkv_dot(j, opq, q_s, 0)
            prep_part(1, opk, ds(j, HD // NT))
            prep_part(2, opv, ds(j, HD // NT))
            layernorm(jnp.minimum(j + 1, NT - 1))

        def kv_pass():
            j = step - (NT + 1)
            for c in cp_rest(j):
                c.wait()
            qkv_dot(j, opk, k_s, HALO)
            qkv_dot(jnp.minimum(j, NT - 1), opv, v_s, HALO)
            prep_rest(j)

        def attention(base, r0):
            def shifted(ref, m):
                kk = ref[pl.ds(base + r0, R + HALO), m * 128:(m + 1) * 128]
                out = [None] * W
                for r in range(4):
                    a = kk[8 - 2 * r: 8 - 2 * r + R + 8]
                    out[r] = a[8:R + 8]
                    out[r + 4] = a[0:R]
                return out
            prods = [[] for _ in range(W)]
            for m in range(8):
                qm = q_s[pl.ds(base + r0, R), m * 128:(m + 1) * 128]
                ks = shifted(k_s, m)
                for w in range(W):
                    prods[w].append(qm * ks[w])
            lane = lax.broadcasted_iota(i32, (R, 128), 1)
            pos = base + r0 + lax.broadcasted_iota(i32, (R, 128), 0)
            logits = []
            for w in range(W):
                l = _tree_sum(prods[w])
                l = l + jnp.take_along_axis(l, lane ^ 1, axis=1)
                l = l + jnp.take_along_axis(l, lane ^ 2, axis=1)
                if w > 0:
                    l = jnp.where(pos >= DIL * w, l, -1e9)
                logits.append(l)
            mx = functools.reduce(jnp.maximum, logits)
            es = [jnp.exp2((l - mx) * exp_c) for l in logits]
            inv = 1.0 / _tree_sum(es)
            a = [e * inv for e in es]
            ot = []
            for m in range(8):
                vs = shifted(v_s, m)
                ot.append(_tree_sum([a[w] * vs[w] for w in range(W)]))
            o_s[pl.ds(r0, R), :] = jnp.concatenate(untwist(ot), axis=1)

        def ffn_pass():
            t = step - (2 * NT + 1)
            base = pl.multiple_of(t * M, M)
            ts = (t, jnp.minimum(t, NT - 1), jnp.maximum(t, 0), jnp.clip(t, 0, NT))
            done = 0
            md = [None] * 7
            for c in range(NC):
                g = combine([dot(load_a(i, ts[(2 * c) % 4]), b_operand(wg_v, wg_e, i, HF, 0, HD, c * CN, CN))
                             for i in range(7)])
                u = combine([dot(load_a(i, ts[(2 * c + 1) % 4]), b_operand(wu_v, wu_e, i, HF, 0, HD, c * CN, CN))
                             for i in range(7)])
                e = a_operands(*[silu(g[i]) * u[i] for i in range(4)])
                for i in range(7):
                    d = dot(e[i], b_operand(wd_v, wd_e, i, HD, c * CN, CN, 0, HD))
                    md[i] = d if md[i] is None else md[i] + d
                tgt = min(NSUB, ((c + 1) * NSUB + NC - 1) // NC)
                while done < tgt:
                    attention(base, done * R)
                    done += 1
            gate = [silu(y) for y in combine(md)]
            oa = a_operands(o_s[0:HM, 0:HD], o_s[0:HM, HD:D], o_s[HM:M, 0:HD], o_s[HM:M, HD:D])
            s = combine([dot(oa[i], b_operand(wo_v, wo_e, i, HD, 0, HD, 0, HD)) for i in range(7)])
            for bi in range(4):
                r0, c0 = (bi // 2) * HM, (bi % 2) * HD
                xr = x_s[pl.ds(base + r0, HM), c0:c0 + HD].astype(f32)
                out_ref[r0:r0 + HM, c0:c0 + HD] = (xr + s[bi] * gate[bi]).astype(out_ref.dtype)

        with scope('pro'):
            pl.when(step == 0)(prologue)
        with scope('Q'):
            pl.when(jnp.logical_and(step >= 1, step <= NT))(q_pass)
        with scope('KV'):
            pl.when(jnp.logical_and(step > NT, step <= 2 * NT))(kv_pass)
        with scope('B'):
            pl.when(step > 2 * NT)(ffn_pass)

    def fn(A_x, A_wqkv, A_wo, B_x, B_w_gate, B_w_up, B_w_down):
        del B_x
        out = pl.pallas_call(
            kernel,
            grid=(3 * NT + 1,),
            in_specs=[pl.BlockSpec(memory_space=pl.ANY)] * 6,
            out_specs=pl.BlockSpec((M, D), lambda s: (jnp.maximum(s - (2 * NT + 1), 0), 0)),
            out_shape=jax.ShapeDtypeStruct((S, D), bf16),
            scratch_shapes=[
                pltpu.VMEM((S, D), bf16),
                pltpu.VMEM((2, HD, 3 * D), bf16), pltpu.VMEM((2, HD, D), bf16),
                pltpu.VMEM((2, HD, F), bf16), pltpu.VMEM((2, HD, F), bf16), pltpu.VMEM((2, HF, D), bf16),
                pltpu.VMEM((7, HD, HD), bf16), pltpu.VMEM((7, HD, HD), bf16), pltpu.VMEM((7, HD, HD), bf16),
                pltpu.VMEM((5, HD, HD), bf16),
                pltpu.VMEM((5, HD, HF), bf16), pltpu.VMEM((5, HD, HF), bf16), pltpu.VMEM((5, HF, HD), bf16),
                pltpu.VMEM((7, S // 4, HD), i32),
                pltpu.VMEM((S, D), f32), pltpu.VMEM((S + HALO, D), f32), pltpu.VMEM((S + HALO, D), f32),
                pltpu.VMEM((M, D), f32),
                pltpu.SemaphoreType.DMA((3 * NT + QC,)),
            ],
            compiler_params=pltpu.CompilerParams(
                dimension_semantics=("arbitrary",), vmem_limit_bytes=vmem_mb * 1024 * 1024, flags=flags),
        )(A_x.reshape(S, D), A_wqkv.reshape(2, HD, 3 * D), A_wo.reshape(2, HD, D), B_w_gate.reshape(2, HD, F),
          B_w_up.reshape(2, HD, F), B_w_down.reshape(2, HF, D))
        return out.reshape(1, S, D)
    return fn

pallas_recurrent_scan__sliding_local_dilated__swiglu_ffn__prompt_kernel = jax.jit(make(rest_early=True))
```

```python
import functools, os, contextlib
import jax
import jax.numpy as jnp
import numpy as np
from jax import lax
import jax.experimental.pallas as pl
import jax.experimental.pallas.tpu as pltpu

S, D, F, H, DH = 2048, 1024, 3584, 32, 32
W, DIL = 8, 2
HALO = 16
HD, HF = D // 2, F // 2
f32, bf16, i32 = jnp.float32, jnp.bfloat16, jnp.int32
scope = (lambda n: jax.named_scope(n)) if os.environ.get('SCOPES') else (lambda n: contextlib.nullcontext())
EVEN = {'XLA_TPU_EVENLY_DISTRIBUTE_CRITICAL_NODES': True}


def _level(a, b, bit, lane):
    lo = (lane & (1 << bit)) == 0
    x = jnp.where(lo, a, b)
    y = jnp.take_along_axis(jnp.where(lo, b, a), lane ^ (1 << bit), axis=1)
    return x, y


def _unlevel(x, y, bit, lane):
    lo = (lane & (1 << bit)) == 0
    yp = jnp.take_along_axis(y, lane ^ (1 << bit), axis=1)
    return jnp.where(lo, x, yp), jnp.where(lo, yp, x)


def twist(c):
    lane = lax.broadcasted_iota(i32, c[0].shape, 1)
    n = [None] * 8
    for p in range(4):
        n[p], n[4 + p] = _level(c[2 * p], c[2 * p + 1], 4, lane)
    c, n = n, [None] * 8
    for g in range(2):
        for p in range(2):
            n[g * 4 + p], n[g * 4 + 2 + p] = _level(c[g * 4 + 2 * p], c[g * 4 + 2 * p + 1], 3, lane)
    c, n = n, [None] * 8
    for g in range(4):
        n[g * 2], n[g * 2 + 1] = _level(c[g * 2], c[g * 2 + 1], 2, lane)
    return n


def untwist(t):
    lane = lax.broadcasted_iota(i32, t[0].shape, 1)
    n = [None] * 8
    for g in range(4):
        n[g * 2], n[g * 2 + 1] = _unlevel(t[g * 2], t[g * 2 + 1], 2, lane)
    c, n = n, [None] * 8
    for g in range(2):
        for p in range(2):
            n[g * 4 + 2 * p], n[g * 4 + 2 * p + 1] = _unlevel(c[g * 4 + p], c[g * 4 + 2 + p], 3, lane)
    c, n = n, [None] * 8
    for p in range(4):
        n[2 * p], n[2 * p + 1] = _unlevel(c[p], c[4 + p], 4, lane)
    return n


def _tree_sum(xs):
    xs = list(xs)
    while len(xs) > 1:
        nxt = [xs[i] + xs[i + 1] for i in range(0, len(xs) - 1, 2)]
        if len(xs) % 2:
            nxt.append(xs[-1])
        xs = nxt
    return xs[0]


def dot(a, b):
    return jnp.dot(a, b, preferred_element_type=f32)


def a_operands(a11, a12, a21, a22):
    return [(a11 + a22).astype(bf16), (a21 + a22).astype(bf16), a11.astype(bf16), a22.astype(bf16),
            (a11 + a12).astype(bf16), (a21 - a11).astype(bf16), (a12 - a22).astype(bf16)]


def combine(m):
    return (m[0] + m[3] - m[4] + m[6], m[2] + m[4], m[1] + m[3], m[0] - m[1] + m[2] + m[5])


def strassen(prod):
    m2, m4 = prod(1), prod(3)
    c21 = m2 + m4
    m3 = prod(2)
    c22 = m3 - m2
    m5 = prod(4)
    c12 = m3 + m5
    c11 = m4 - m5
    m1 = prod(0)
    c11 = c11 + m1 + prod(6)
    c22 = c22 + m1 + prod(5)
    return c11, c12, c21, c22


def quarters(x):
    hm, hk = x.shape[0] // 2, x.shape[1] // 2
    return x[:hm, :hk], x[:hm, hk:], x[hm:, :hk], x[hm:, hk:]


def b_operand(raw, ext, i, hn, k0, kn, n0, nn):
    if i in (1, 4):
        r = 0 if i == 1 else 1
        return raw[r, k0:k0 + kn, r * hn + n0:r * hn + n0 + nn]
    return ext[{0: 0, 2: 1, 3: 2, 5: 3, 6: 4}[i], k0:k0 + kn, n0:n0 + nn]


def b_sums(b11, b12, b21, b22):
    b11, b12, b21, b22 = [b.astype(f32) for b in (b11, b12, b21, b22)]
    return [(b11 + b22).astype(bf16), (b12 - b22).astype(bf16), (b21 - b11).astype(bf16),
            (b11 + b12).astype(bf16), (b21 + b22).astype(bf16)]


def make(M=256, CN=1792, R=16, vmem_mb=120, flags=EVEN, RB=16, CB=256, QC=4, anchor=True, rest_early=True, a_first=False, LG=16, NB=128, border=False, NF=None):
    NF = NF or CN
    NT = S // M
    HM = M // 2
    NC = HF // CN
    NSUB = M // R
    exp_c = float(DH ** -0.5 * np.log2(np.e))
    SX, SQ, SKV, SR = 0, NT, NT + QC, 2 * NT + QC

    def silu(g):
        hg = 0.5 * g
        return hg * jnp.tanh(hg) + hg

    def kernel(x_h, wqkv_h, wo_h, wg_h, wu_h, wd_h, out_ref,
               x_s, wqkv_v, wo_v, wg_v, wu_v, wd_v, opq, opk, opv, wo_e, wg_e, wu_e, wd_e,
               xa_s, q_s, k_s, v_s, o_s, sems):
        step = pl.program_id(0)
        zero = jnp.minimum(step, 0)

        def ds(i, n):
            return pl.ds(pl.multiple_of(i * n, n), n)

        def cp_x(t):
            return pltpu.make_async_copy(x_h.at[ds(t, M), :], x_s.at[ds(t, M), :], sems.at[SX + t])

        def cp_w(p, rows, sem):
            return pltpu.make_async_copy(wqkv_h.at[:, rows, pl.ds(p * D, D)], wqkv_v.at[:, rows, pl.ds(p * D, D)],
                                         sems.at[sem])

        def cp_q(r):
            return cp_w(0, ds(r, HD // QC), SQ + r)

        def cp_kv(j):
            return [cp_w(p, ds(j, HD // NT), SKV + j) for p in (1, 2)]

        rest = [(wg_h, wg_v, wg_e, HD // NT, HF), (wu_h, wu_v, wu_e, HD // NT, HF),
                (wd_h, wd_v, wd_e, HF // NT, HD), (wo_h, wo_v, wo_e, HD // NT, HD)]

        def cp_rest(j):
            return [pltpu.make_async_copy(src.at[:, ds(j, n), :], raw.at[:, ds(j, n), :], sems.at[SR + j])
                    for src, raw, _, n, _ in rest]

        def layernorm(t):
            def norm(r0):
                x = x_s[pl.ds(pl.multiple_of(t * M + r0, LG), LG), :].astype(f32)
                xc = x - jnp.mean(x, axis=-1, keepdims=True)
                return xc * lax.rsqrt(jnp.mean(xc * xc, axis=-1, keepdims=True) + 1e-5)
            for r in range(0, HM, LG):
                top, bot = norm(r), norm(HM + r)
                a = a_operands(top[:, :HD], top[:, HD:], bot[:, :HD], bot[:, HD:])
                for i in range(7):
                    xa_s[i, pl.ds(pl.multiple_of(t * (HM // 2) + r // 2, LG // 2), LG // 2), :] = pltpu.bitcast(a[i], i32)

        def load_a(i, t):
            return pltpu.bitcast(xa_s[i, ds(t, HM // 2), :], bf16)

        def prep_part(p, op, rows):
            blk = []
            for half in range(2):
                w = pltpu.bitcast(wqkv_v[half, rows, pl.ds(p * D, D)], i32)
                t = twist([w[:, c * 128:(c + 1) * 128] for c in range(8)])
                blk += [pltpu.bitcast(jnp.concatenate(t[:4], axis=1), bf16),
                        pltpu.bitcast(jnp.concatenate(t[4:], axis=1), bf16)]
            e = b_sums(*blk)
            for i, v in zip((0, 2, 3, 5, 6, 1, 4), e + [blk[0], blk[3]]):
                op[i, rows, :] = v

        def prep_rest(j):
            for _, raw, ext, n, hn in rest:
                for r in range(0, n, RB):
                    rows = pl.ds(pl.multiple_of(j * n + r, RB), RB)
                    for c in range(0, hn, CB):
                        b11, b22 = raw[0, rows, c:c + CB], raw[1, rows, hn + c:hn + c + CB]
                        if anchor:
                            b11, b22 = [jnp.concatenate(
                                [pltpu.bitcast(pltpu.roll(pltpu.bitcast(b[:, k:k + 128], i32), zero, 1), bf16)
                                 for k in range(0, CB, 128)], axis=1) for b in (b11, b22)]
                        e = b_sums(b11, raw[0, rows, hn + c:hn + c + CB], raw[1, rows, c:c + CB], b22)
                        for i in range(5):
                            ext[i, rows, c:c + CB] = e[i]

        def qkv_dot(t, op, dst, off, a=None):
            ts = (t, jnp.minimum(t, NT - 1), jnp.maximum(t, 0), jnp.clip(t, 0, NT))
            for n, n0 in enumerate(range(0, HD, NB)):
                c = strassen(lambda i: dot(load_a(i, ts[n % 4]), op[i, :, n0:n0 + NB]))
                for bi, blk in enumerate(c):
                    dst[pl.ds(pl.multiple_of(t * M, M) + off + (bi // 2) * HM, HM),
                        (bi % 2) * HD + n0:(bi % 2) * HD + n0 + NB] = blk

        def prologue():
            cp_x(0).start()
            for r in range(QC):
                cp_q(r).start()

            def start_kv(j, carry):
                @pl.when(j < NT - 1)
                def _():
                    cp_x(j + 1).start()
                for c in cp_kv(j):
                    c.start()
                return carry
            lax.fori_loop(0, NT, start_kv, 0)
            if rest_early:
                def start_rest(j, carry):
                    for c in cp_rest(j):
                        c.start()
                    return carry
                lax.fori_loop(0, NT, start_rest, 0)
            k_s[pl.ds(0, HALO), :] = jnp.zeros((HALO, D), f32)
            v_s[pl.ds(0, HALO), :] = jnp.zeros((HALO, D), f32)
            cp_x(0).wait()
            layernorm(0)

            def prep_q(r, carry):
                cp_q(r).wait()
                prep_part(0, opq, ds(r, HD // QC))
                return carry
            lax.fori_loop(0, QC, prep_q, 0)

        def q_pass():
            j = step - 1
            if not rest_early:
                for c in cp_rest(j):
                    c.start()

            @pl.when(j < NT - 1)
            def _():
                cp_x(j + 1).wait()
            for c in cp_kv(j):
                c.wait()
            if a_first:
                a = [load_a(i, j) for i in range(7)]
                layernorm(jnp.minimum(j + 1, NT - 1))
                qkv_dot(j, opq, q_s, 0, a)
            else:
                qkv_dot(j, opq, q_s, 0)
            prep_part(1, opk, ds(j, HD // NT))
            prep_part(2, opv, ds(j, HD // NT))
            if not a_first:
                layernorm(jnp.minimum(j + 1, NT - 1))

        def kv_pass():
            j = step - (NT + 1)
            for c in cp_rest(j):
                c.wait()
            qkv_dot(j, opk, k_s, HALO)
            qkv_dot(jnp.minimum(j, NT - 1), opv, v_s, HALO)
            prep_rest(j)

        def attention(base, r0):
            def shifted(ref, m):
                kk = ref[pl.ds(base + r0, R + HALO), m * 128:(m + 1) * 128]
                out = [None] * W
                for r in range(4):
                    a = kk[8 - 2 * r: 8 - 2 * r + R + 8]
                    out[r] = a[8:R + 8]
                    out[r + 4] = a[0:R]
                return out
            prods = [[] for _ in range(W)]
            for m in range(8):
                qm = q_s[pl.ds(base + r0, R), m * 128:(m + 1) * 128]
                ks = shifted(k_s, m)
                for w in range(W):
                    prods[w].append(qm * ks[w])
            lane = lax.broadcasted_iota(i32, (R, 128), 1)
            pos = base + r0 + lax.broadcasted_iota(i32, (R, 128), 0)
            logits = []
            for w in range(W):
                l = _tree_sum(prods[w])
                l = l + jnp.take_along_axis(l, lane ^ 1, axis=1)
                l = l + jnp.take_along_axis(l, lane ^ 2, axis=1)
                if w > 0:
                    l = jnp.where(pos >= DIL * w, l, -1e9)
                logits.append(l)
            mx = functools.reduce(jnp.maximum, logits)
            es = [jnp.exp2((l - mx) * exp_c) for l in logits]
            inv = 1.0 / _tree_sum(es)
            a = [e * inv for e in es]
            ot = []
            for m in range(8):
                vs = shifted(v_s, m)
                ot.append(_tree_sum([a[w] * vs[w] for w in range(W)]))
            o_s[pl.ds(r0, R), :] = jnp.concatenate(untwist(ot), axis=1)

        def ffn_pass():
            t = step - (2 * NT + 1)
            base = pl.multiple_of(t * M, M)
            ts = (t, jnp.minimum(t, NT - 1), jnp.maximum(t, 0), jnp.clip(t, 0, NT))
            done = 0
            md = [None] * 7
            nld = 0
            for c in range(NC):
                pieces = []
                for n0 in range(c * CN, (c + 1) * CN, NF):
                    def prod(raw, ext, i):
                        return dot(load_a(i, ts[(nld + (raw is wg_v)) % 4]), b_operand(raw, ext, i, HF, 0, HD, n0, NF))
                    comb = strassen if border else (lambda f: combine([f(i) for i in range(7)]))
                    g = comb(functools.partial(prod, wg_v, wg_e))
                    u = comb(functools.partial(prod, wu_v, wu_e))
                    nld += 2
                    pieces.append(a_operands(*[silu(g[i]) * u[i] for i in range(4)]))
                    tgt = min(NSUB, ((n0 + NF) * NSUB + HF - 1) // HF)
                    while done < tgt:
                        attention(base, done * R)
                        done += 1
                for i in range(7):
                    e = pieces[0][i] if len(pieces) == 1 else jnp.concatenate([p[i] for p in pieces], axis=1)
                    d = dot(e, b_operand(wd_v, wd_e, i, HD, c * CN, CN, 0, HD))
                    md[i] = d if md[i] is None else md[i] + d
            gate = [silu(y) for y in combine(md)]
            oa = a_operands(o_s[0:HM, 0:HD], o_s[0:HM, HD:D], o_s[HM:M, 0:HD], o_s[HM:M, HD:D])
            s = combine([dot(oa[i], b_operand(wo_v, wo_e, i, HD, 0, HD, 0, HD)) for i in range(7)])
            for bi in range(4):
                r0, c0 = (bi // 2) * HM, (bi % 2) * HD
                xr = x_s[pl.ds(base + r0, HM), c0:c0 + HD].astype(f32)
                out_ref[r0:r0 + HM, c0:c0 + HD] = (xr + s[bi] * gate[bi]).astype(out_ref.dtype)

        with scope('pro'):
            pl.when(step == 0)(prologue)
        with scope('Q'):
            pl.when(jnp.logical_and(step >= 1, step <= NT))(q_pass)
        with scope('KV'):
            pl.when(jnp.logical_and(step > NT, step <= 2 * NT))(kv_pass)
        with scope('B'):
            pl.when(step > 2 * NT)(ffn_pass)

    def fn(A_x, A_wqkv, A_wo, B_x, B_w_gate, B_w_up, B_w_down):
        del B_x
        out = pl.pallas_call(
            kernel,
            grid=(3 * NT + 1,),
            in_specs=[pl.BlockSpec(memory_space=pl.ANY)] * 6,
            out_specs=pl.BlockSpec((M, D), lambda s: (jnp.maximum(s - (2 * NT + 1), 0), 0)),
            out_shape=jax.ShapeDtypeStruct((S, D), bf16),
            scratch_shapes=[
                pltpu.VMEM((S, D), bf16),
                pltpu.VMEM((2, HD, 3 * D), bf16), pltpu.VMEM((2, HD, D), bf16),
                pltpu.VMEM((2, HD, F), bf16), pltpu.VMEM((2, HD, F), bf16), pltpu.VMEM((2, HF, D), bf16),
                pltpu.VMEM((7, HD, HD), bf16), pltpu.VMEM((7, HD, HD), bf16), pltpu.VMEM((7, HD, HD), bf16),
                pltpu.VMEM((5, HD, HD), bf16),
                pltpu.VMEM((5, HD, HF), bf16), pltpu.VMEM((5, HD, HF), bf16), pltpu.VMEM((5, HF, HD), bf16),
                pltpu.VMEM((7, S // 4, HD), i32),
                pltpu.VMEM((S, D), f32), pltpu.VMEM((S + HALO, D), f32), pltpu.VMEM((S + HALO, D), f32),
                pltpu.VMEM((M, D), f32),
                pltpu.SemaphoreType.DMA((3 * NT + QC,)),
            ],
            compiler_params=pltpu.CompilerParams(
                dimension_semantics=("arbitrary",), vmem_limit_bytes=vmem_mb * 1024 * 1024, flags=flags),
        )(A_x.reshape(S, D), A_wqkv.reshape(2, HD, 3 * D), A_wo.reshape(2, HD, D), B_w_gate.reshape(2, HD, F),
          B_w_up.reshape(2, HD, F), B_w_down.reshape(2, HF, D))
        return out.reshape(1, S, D)
    return fn

pallas_recurrent_scan__sliding_local_dilated__swiglu_ffn__prompt_kernel = jax.jit(make())
```

```python
import functools

import jax
from jax import lax
import jax.experimental.pallas as pl
import jax.experimental.pallas.tpu as pltpu
import jax.numpy as jnp
import numpy as np

S, D, F = 2048, 1024, 3584
DH, W, DIL = 32, 8, 2
HALO = 16
HD, HF = D // 2, F // 2
M = 256
HM = M // 2
NT = S // M
R = 16
LG = 16
NB = 128
NO = 512
QC = 4
RB, CB = 16, 256
EXP_C = float(DH ** -0.5 * np.log2(np.e))
SEM_X, SEM_Q, SEM_KV, SEM_REST = 0, NT, NT + QC, 2 * NT + QC
NSEM = 3 * NT + QC

f32, bf16, i32 = jnp.float32, jnp.bfloat16, jnp.int32


def _twist_level(a, b, bit, lane):
    lo = (lane & (1 << bit)) == 0
    return jnp.where(lo, a, b), jnp.take_along_axis(jnp.where(lo, b, a), lane ^ (1 << bit), axis=1)


def _untwist_level(x, y, bit, lane):
    lo = (lane & (1 << bit)) == 0
    yp = jnp.take_along_axis(y, lane ^ (1 << bit), axis=1)
    return jnp.where(lo, x, yp), jnp.where(lo, yp, x)


def _twist(c):
    lane = lax.broadcasted_iota(i32, c[0].shape, 1)
    n = [None] * 8
    for p in range(4):
        n[p], n[4 + p] = _twist_level(c[2 * p], c[2 * p + 1], 4, lane)
    c, n = n, [None] * 8
    for g in range(0, 8, 4):
        for p in range(2):
            n[g + p], n[g + 2 + p] = _twist_level(c[g + 2 * p], c[g + 2 * p + 1], 3, lane)
    c, n = n, [None] * 8
    for g in range(0, 8, 2):
        n[g], n[g + 1] = _twist_level(c[g], c[g + 1], 2, lane)
    return n


def _untwist(c):
    lane = lax.broadcasted_iota(i32, c[0].shape, 1)
    n = [None] * 8
    for g in range(0, 8, 2):
        n[g], n[g + 1] = _untwist_level(c[g], c[g + 1], 2, lane)
    c, n = n, [None] * 8
    for g in range(0, 8, 4):
        for p in range(2):
            n[g + 2 * p], n[g + 2 * p + 1] = _untwist_level(c[g + p], c[g + 2 + p], 3, lane)
    c, n = n, [None] * 8
    for p in range(4):
        n[2 * p], n[2 * p + 1] = _untwist_level(c[p], c[4 + p], 4, lane)
    return n


def _dot(a, b):
    return jnp.dot(a, b, preferred_element_type=f32)


def _left(a11, a12, a21, a22):
    return [(a11 + a22).astype(bf16), (a21 + a22).astype(bf16), a11.astype(bf16), a22.astype(bf16),
            (a11 + a12).astype(bf16), (a21 - a11).astype(bf16), (a12 - a22).astype(bf16)]


def _right_sums(b11, b12, b21, b22):
    b11, b12, b21, b22 = [b.astype(f32) for b in (b11, b12, b21, b22)]
    return [(b11 + b22).astype(bf16), (b12 - b22).astype(bf16), (b21 - b11).astype(bf16),
            (b11 + b12).astype(bf16), (b21 + b22).astype(bf16)]


def _right(raw, ext, i, hn, k0, kn, n0, nn):
    if i in (1, 4):
        r = 0 if i == 1 else 1
        return raw[r, k0:k0 + kn, r * hn + n0:r * hn + n0 + nn]
    return ext[{0: 0, 2: 1, 3: 2, 5: 3, 6: 4}[i], k0:k0 + kn, n0:n0 + nn]


def _strassen(prod):
    m2, m4 = prod(1), prod(3)
    c21 = m2 + m4
    m3 = prod(2)
    c22 = m3 - m2
    m5 = prod(4)
    c12 = m3 + m5
    c11 = m4 - m5
    m1 = prod(0)
    c11 = c11 + m1 + prod(6)
    c22 = c22 + m1 + prod(5)
    return c11, c12, c21, c22


def _combine(m):
    return m[0] + m[3] - m[4] + m[6], m[2] + m[4], m[1] + m[3], m[0] - m[1] + m[2] + m[5]


def _tree_sum(xs):
    xs = list(xs)
    while len(xs) > 1:
        xs = [xs[i] + xs[i + 1] for i in range(0, len(xs), 2)]
    return xs[0]


def _silu(g):
    hg = 0.5 * g
    return hg * jnp.tanh(hg) + hg


def _ds(i, n):
    return pl.ds(pl.multiple_of(i * n, n), n)


def _same(t):
    return t, jnp.minimum(t, NT - 1), jnp.maximum(t, 0), jnp.clip(t, 0, NT)


def _kernel(x_h, wqkv_h, wo_h, wg_h, wu_h, wd_h, out_ref,
            x_s, wqkv_v, wo_v, wg_v, wu_v, wd_v, opq, opk, opv, wo_e, wg_e, wu_e, wd_e,
            xa_s, q_s, k_s, v_s, o_s, sems):
    step = pl.program_id(0)
    zero = jnp.minimum(step, 0)

    def cp_x(t):
        return pltpu.make_async_copy(x_h.at[_ds(t, M), :], x_s.at[_ds(t, M), :], sems.at[SEM_X + t])

    def cp_w(p, rows, sem):
        return pltpu.make_async_copy(wqkv_h.at[:, rows, pl.ds(p * D, D)], wqkv_v.at[:, rows, pl.ds(p * D, D)],
                                     sems.at[sem])

    def cp_q(r):
        return cp_w(0, _ds(r, HD // QC), SEM_Q + r)

    def cp_kv(j):
        return [cp_w(p, _ds(j, HD // NT), SEM_KV + j) for p in (1, 2)]

    rest = [(wg_h, wg_v, wg_e, HD // NT, HF), (wu_h, wu_v, wu_e, HD // NT, HF),
            (wd_h, wd_v, wd_e, HF // NT, HD), (wo_h, wo_v, wo_e, HD // NT, HD)]

    def cp_rest(j):
        return [pltpu.make_async_copy(src.at[:, _ds(j, n), :], raw.at[:, _ds(j, n), :], sems.at[SEM_REST + j])
                for src, raw, _, n, _ in rest]

    def layernorm(t):
        def norm(r0):
            x = x_s[pl.ds(pl.multiple_of(t * M + r0, LG), LG), :].astype(f32)
            xc = x - jnp.mean(x, axis=-1, keepdims=True)
            return xc * lax.rsqrt(jnp.mean(xc * xc, axis=-1, keepdims=True) + 1e-5)
        for r in range(0, HM, LG):
            top, bot = norm(r), norm(HM + r)
            a = _left(top[:, :HD], top[:, HD:], bot[:, :HD], bot[:, HD:])
            for i in range(7):
                xa_s[i, pl.ds(pl.multiple_of(t * (HM // 2) + r // 2, LG // 2), LG // 2), :] = pltpu.bitcast(a[i], i32)

    def load_a(i, t):
        return pltpu.bitcast(xa_s[i, _ds(t, HM // 2), :], bf16)

    def prep_part(p, op, rows):
        blk = []
        for half in range(2):
            w = pltpu.bitcast(wqkv_v[half, rows, pl.ds(p * D, D)], i32)
            t = _twist([w[:, c * 128:(c + 1) * 128] for c in range(8)])
            blk += [pltpu.bitcast(jnp.concatenate(t[:4], axis=1), bf16),
                    pltpu.bitcast(jnp.concatenate(t[4:], axis=1), bf16)]
        for i, v in zip((0, 2, 3, 5, 6, 1, 4), _right_sums(*blk) + [blk[0], blk[3]]):
            op[i, rows, :] = v

    def prep_rest(j):
        def pass_through_xlu(b):
            return jnp.concatenate([pltpu.bitcast(pltpu.roll(pltpu.bitcast(b[:, k:k + 128], i32), zero, 1), bf16)
                                    for k in range(0, CB, 128)], axis=1)
        for _, raw, ext, n, hn in rest:
            for r in range(0, n, RB):
                rows = pl.ds(pl.multiple_of(j * n + r, RB), RB)
                for c in range(0, hn, CB):
                    e = _right_sums(pass_through_xlu(raw[0, rows, c:c + CB]), raw[0, rows, hn + c:hn + c + CB],
                                    raw[1, rows, c:c + CB], pass_through_xlu(raw[1, rows, hn + c:hn + c + CB]))
                    for i in range(5):
                        ext[i, rows, c:c + CB] = e[i]

    def qkv_dot(t, op, dst, off):
        ts = _same(t)
        for n, n0 in enumerate(range(0, HD, NB)):
            c = _strassen(lambda i: _dot(load_a(i, ts[n % 4]), op[i, :, n0:n0 + NB]))
            for bi, blk in enumerate(c):
                dst[pl.ds(pl.multiple_of(t * M, M) + off + (bi // 2) * HM, HM),
                    (bi % 2) * HD + n0:(bi % 2) * HD + n0 + NB] = blk

    def prologue():
        cp_x(0).start()
        for r in range(QC):
            cp_q(r).start()

        def start_kv(j, carry):
            @pl.when(j < NT - 1)
            def _():
                cp_x(jnp.minimum(j + 1, NT - 1)).start()
            for c in cp_kv(j):
                c.start()
            return carry
        lax.fori_loop(0, NT, start_kv, 0)

        def start_rest(j, carry):
            for c in cp_rest(j):
                c.start()
            return carry
        lax.fori_loop(0, NT, start_rest, 0)
        k_s[pl.ds(0, HALO), :] = jnp.zeros((HALO, D), f32)
        v_s[pl.ds(0, HALO), :] = jnp.zeros((HALO, D), f32)
        cp_x(0).wait()
        layernorm(0)

        def prep_q(r, carry):
            cp_q(r).wait()
            prep_part(0, opq, _ds(r, HD // QC))
            return carry
        lax.fori_loop(0, QC, prep_q, 0)

    def q_pass():
        j = step - 1
        nxt = jnp.minimum(j + 1, NT - 1)

        @pl.when(j < NT - 1)
        def _():
            cp_x(nxt).wait()
        for c in cp_kv(j):
            c.wait()
        qkv_dot(j, opq, q_s, 0)
        prep_part(1, opk, _ds(j, HD // NT))
        prep_part(2, opv, _ds(j, HD // NT))
        layernorm(nxt)

    def kv_pass():
        j = step - (NT + 1)
        for c in cp_rest(j):
            c.wait()
        qkv_dot(j, opk, k_s, HALO)
        qkv_dot(jnp.minimum(j, NT - 1), opv, v_s, HALO)
        prep_rest(j)

    def attention(base, r0):
        def taps(ref, m):
            kk = ref[pl.ds(base + r0, R + HALO), m * 128:(m + 1) * 128]
            out = [None] * W
            for r in range(4):
                a = kk[8 - DIL * r:8 - DIL * r + R + 8]
                out[r], out[r + 4] = a[8:R + 8], a[0:R]
            return out
        prods = [[] for _ in range(W)]
        for m in range(8):
            qm = q_s[pl.ds(base + r0, R), m * 128:(m + 1) * 128]
            km = taps(k_s, m)
            for w in range(W):
                prods[w].append(qm * km[w])
        lane = lax.broadcasted_iota(i32, (R, 128), 1)
        pos = base + r0 + lax.broadcasted_iota(i32, (R, 128), 0)
        logits = []
        for w in range(W):
            l = _tree_sum(prods[w])
            l = l + jnp.take_along_axis(l, lane ^ 1, axis=1)
            l = l + jnp.take_along_axis(l, lane ^ 2, axis=1)
            if w > 0:
                l = jnp.where(pos >= DIL * w, l, -1e9)
            logits.append(l)
        mx = functools.reduce(jnp.maximum, logits)
        es = [jnp.exp2((l - mx) * EXP_C) for l in logits]
        inv = 1.0 / _tree_sum(es)
        a = [e * inv for e in es]
        ot = []
        for m in range(8):
            vm = taps(v_s, m)
            ot.append(_tree_sum([a[w] * vm[w] for w in range(W)]))
        o_s[pl.ds(r0, R), :] = jnp.concatenate(_untwist(ot), axis=1)

    def ffn_pass():
        t = step - (2 * NT + 1)
        base = pl.multiple_of(t * M, M)
        ts = _same(t)
        g = _combine([_dot(load_a(i, ts[0]), _right(wg_v, wg_e, i, HF, 0, HD, 0, HF)) for i in range(7)])
        u = _combine([_dot(load_a(i, ts[1]), _right(wu_v, wu_e, i, HF, 0, HD, 0, HF)) for i in range(7)])
        e = _left(*[_silu(g[i]) * u[i] for i in range(4)])
        for r0 in range(0, M, R):
            attention(base, r0)
        md = [_dot(e[i], _right(wd_v, wd_e, i, HD, 0, HF, 0, HD)) for i in range(7)]
        gate = [_silu(y) for y in _combine(md)]
        oa = _left(o_s[0:HM, 0:HD], o_s[0:HM, HD:D], o_s[HM:M, 0:HD], o_s[HM:M, HD:D])
        for n0 in range(0, HD, NO):
            s = _strassen(lambda i: _dot(oa[i], _right(wo_v, wo_e, i, HD, 0, HD, n0, NO)))
            for bi in range(4):
                r0, c0 = (bi // 2) * HM, (bi % 2) * HD + n0
                xr = x_s[pl.ds(base + r0, HM), c0:c0 + NO].astype(f32)
                out_ref[r0:r0 + HM, c0:c0 + NO] = (xr + s[bi] * gate[bi][:, n0:n0 + NO]).astype(out_ref.dtype)

    pl.when(step == 0)(prologue)
    pl.when(jnp.logical_and(step >= 1, step <= NT))(q_pass)
    pl.when(jnp.logical_and(step > NT, step <= 2 * NT))(kv_pass)
    pl.when(step > 2 * NT)(ffn_pass)


@jax.jit
def pallas_recurrent_scan__sliding_local_dilated__swiglu_ffn__prompt_kernel(
    A_x: jax.Array,
    A_wqkv: jax.Array,
    A_wo: jax.Array,
    B_x: jax.Array,
    B_w_gate: jax.Array,
    B_w_up: jax.Array,
    B_w_down: jax.Array,
):
    del B_x
    out = pl.pallas_call(
        _kernel,
        grid=(3 * NT + 1,),
        in_specs=[pl.BlockSpec(memory_space=pl.ANY)] * 6,
        out_specs=pl.BlockSpec((M, D), lambda s: (jnp.maximum(s - (2 * NT + 1), 0), 0)),
        out_shape=jax.ShapeDtypeStruct((S, D), bf16),
        scratch_shapes=[
            pltpu.VMEM((S, D), bf16),
            pltpu.VMEM((2, HD, 3 * D), bf16), pltpu.VMEM((2, HD, D), bf16),
            pltpu.VMEM((2, HD, F), bf16), pltpu.VMEM((2, HD, F), bf16), pltpu.VMEM((2, HF, D), bf16),
            pltpu.VMEM((7, HD, HD), bf16), pltpu.VMEM((7, HD, HD), bf16), pltpu.VMEM((7, HD, HD), bf16),
            pltpu.VMEM((5, HD, HD), bf16),
            pltpu.VMEM((5, HD, HF), bf16), pltpu.VMEM((5, HD, HF), bf16), pltpu.VMEM((5, HF, HD), bf16),
            pltpu.VMEM((7, S // 4, HD), i32),
            pltpu.VMEM((S, D), f32), pltpu.VMEM((S + HALO, D), f32), pltpu.VMEM((S + HALO, D), f32),
            pltpu.VMEM((M, D), f32),
            pltpu.SemaphoreType.DMA((NSEM,)),
        ],
        compiler_params=pltpu.CompilerParams(
            dimension_semantics=("arbitrary",),
            vmem_limit_bytes=120 * 1024 * 1024,
            flags={"XLA_TPU_EVENLY_DISTRIBUTE_CRITICAL_NODES": True},
        ),
    )(A_x.reshape(S, D), A_wqkv.reshape(2, HD, 3 * D), A_wo.reshape(2, HD, D), B_w_gate.reshape(2, HD, F),
      B_w_up.reshape(2, HD, F), B_w_down.reshape(2, HF, D))
    return out.reshape(1, S, D)
```

```python
import functools

import jax
from jax import lax
import jax.experimental.pallas as pl
import jax.experimental.pallas.tpu as pltpu
import jax.numpy as jnp
import numpy as np

S, D, F = 2048, 1024, 3584
DH, W, DIL = 32, 8, 2
HALO = 16
HD, HF = D // 2, F // 2
M = 256
HM = M // 2
NT = S // M
R = 16
LG = 16
NB = 128
NO = 512
QC = 4
RB, CB = 16, 256
EXP_C = float(DH ** -0.5 * np.log2(np.e))
SEM_X, SEM_Q, SEM_KV, SEM_REST, SEM_OUT = 0, NT, NT + QC, 2 * NT + QC, 3 * NT + QC
NSEM = 3 * NT + QC + 2

f32, bf16, i32 = jnp.float32, jnp.bfloat16, jnp.int32


def _twist_level(a, b, bit, lane):
    lo = (lane & (1 << bit)) == 0
    return jnp.where(lo, a, b), jnp.take_along_axis(jnp.where(lo, b, a), lane ^ (1 << bit), axis=1)


def _untwist_level(x, y, bit, lane):
    lo = (lane & (1 << bit)) == 0
    yp = jnp.take_along_axis(y, lane ^ (1 << bit), axis=1)
    return jnp.where(lo, x, yp), jnp.where(lo, yp, x)


def _twist(c):
    lane = lax.broadcasted_iota(i32, c[0].shape, 1)
    n = [None] * 8
    for p in range(4):
        n[p], n[4 + p] = _twist_level(c[2 * p], c[2 * p + 1], 4, lane)
    c, n = n, [None] * 8
    for g in range(0, 8, 4):
        for p in range(2):
            n[g + p], n[g + 2 + p] = _twist_level(c[g + 2 * p], c[g + 2 * p + 1], 3, lane)
    c, n = n, [None] * 8
    for g in range(0, 8, 2):
        n[g], n[g + 1] = _twist_level(c[g], c[g + 1], 2, lane)
    return n


def _untwist(c):
    lane = lax.broadcasted_iota(i32, c[0].shape, 1)
    n = [None] * 8
    for g in range(0, 8, 2):
        n[g], n[g + 1] = _untwist_level(c[g], c[g + 1], 2, lane)
    c, n = n, [None] * 8
    for g in range(0, 8, 4):
        for p in range(2):
            n[g + 2 * p], n[g + 2 * p + 1] = _untwist_level(c[g + p], c[g + 2 + p], 3, lane)
    c, n = n, [None] * 8
    for p in range(4):
        n[2 * p], n[2 * p + 1] = _untwist_level(c[p], c[4 + p], 4, lane)
    return n


def _dot(a, b):
    return jnp.dot(a, b, preferred_element_type=f32)


def _left_f32(a11, a12, a21, a22):
    return [a11 + a22, a21 + a22, a11, a22, a11 + a12, a21 - a11, a12 - a22]


def _left(*blocks):
    return [a.astype(bf16) for a in _left_f32(*blocks)]


def _right_sums(b11, b12, b21, b22):
    b11, b12, b21, b22 = [b.astype(f32) for b in (b11, b12, b21, b22)]
    return [pltpu.bitcast(v.astype(bf16), i32) for v in (b11 + b22, b12 - b22, b21 - b11, b11 + b12, b21 + b22)]


def _right(raw, ext, i, hn, k0, kn, n0, nn):
    if i in (1, 4):
        r = 0 if i == 1 else 1
        return raw[r, k0:k0 + kn, r * hn + n0:r * hn + n0 + nn]
    e = {0: 0, 2: 1, 3: 2, 5: 3, 6: 4}[i]
    return pltpu.bitcast(ext[e, k0 // 2:(k0 + kn) // 2, n0:n0 + nn], bf16)


def _strassen(prod):
    m2, m4 = prod(1), prod(3)
    c21 = m2 + m4
    m3 = prod(2)
    c22 = m3 - m2
    m5 = prod(4)
    c12 = m3 + m5
    c11 = m4 - m5
    m1 = prod(0)
    c11 = c11 + m1 + prod(6)
    c22 = c22 + m1 + prod(5)
    return c11, c12, c21, c22


def _combine(m):
    return m[0] + m[3] - m[4] + m[6], m[2] + m[4], m[1] + m[3], m[0] - m[1] + m[2] + m[5]


def _tree_sum(xs):
    xs = list(xs)
    while len(xs) > 1:
        xs = [xs[i] + xs[i + 1] for i in range(0, len(xs), 2)]
    return xs[0]


def _silu(g):
    hg = 0.5 * g
    return hg * jnp.tanh(hg) + hg


def _ds(i, n):
    return pl.ds(pl.multiple_of(i * n, n), n)


def _same(t):
    return t, jnp.minimum(t, NT - 1), jnp.maximum(t, 0), jnp.clip(t, 0, NT)


def _kernel(x_h, wqkv_h, wo_h, wg_h, wu_h, wd_h, out_h,
            x_s, wqkv_v, wo_v, wg_v, wu_v, wd_v, opq, opk, opv, wo_e, wg_e, wu_e, wd_e,
            xa_s, q_s, k_s, v_s, o_s, out_s, zero_s, sems):

    def cp_x(t):
        return pltpu.make_async_copy(x_h.at[_ds(t, M), :], x_s.at[_ds(t, M), :], sems.at[SEM_X + t])

    def cp_w(p, rows, sem):
        return pltpu.make_async_copy(wqkv_h.at[:, rows, pl.ds(p * D, D)], wqkv_v.at[:, rows, pl.ds(p * D, D)],
                                     sems.at[sem])

    def cp_q(r):
        return cp_w(0, _ds(r, HD // QC), SEM_Q + r)

    def cp_kv(j):
        return [cp_w(p, _ds(j, HD // NT), SEM_KV + j) for p in (1, 2)]

    rest = [(wg_h, wg_v, wg_e, HD // NT, HF), (wu_h, wu_v, wu_e, HD // NT, HF),
            (wd_h, wd_v, wd_e, HF // NT, HD), (wo_h, wo_v, wo_e, HD // NT, HD)]

    def cp_rest(j):
        return [pltpu.make_async_copy(src.at[:, _ds(j, n), :], raw.at[:, _ds(j, n), :], sems.at[SEM_REST + j])
                for src, raw, _, n, _ in rest]

    def layernorm(t):
        def norm(r0):
            x = x_s[pl.ds(pl.multiple_of(t * M + r0, LG), LG), :].astype(f32)
            xc = x - jnp.mean(x, axis=-1, keepdims=True)
            return xc * lax.rsqrt(jnp.mean(xc * xc, axis=-1, keepdims=True) + 1e-5)
        for r in range(0, HM, LG):
            top, bot = norm(r), norm(HM + r)
            a = _left(top[:, :HD], top[:, HD:], bot[:, :HD], bot[:, HD:])
            for i in range(7):
                xa_s[i, pl.ds(pl.multiple_of(t * (HM // 2) + r // 2, LG // 2), LG // 2), :] = pltpu.bitcast(a[i], i32)

    def load_a(i, t):
        return pltpu.bitcast(xa_s[i, _ds(t, HM // 2), :], bf16)

    def prep_part(p, op, r, n):
        rows, wrows = _ds(r, n), _ds(r, n // 2)
        blk = []
        for half in range(2):
            w = pltpu.bitcast(wqkv_v[half, rows, pl.ds(p * D, D)], i32)
            t = _twist([w[:, c * 128:(c + 1) * 128] for c in range(8)])
            blk += [jnp.concatenate(t[:4], axis=1), jnp.concatenate(t[4:], axis=1)]
        sums = _right_sums(*[pltpu.bitcast(b, bf16) for b in blk])
        for i, v in zip((0, 2, 3, 5, 6, 1, 4), sums + [blk[0], blk[3]]):
            op[i, wrows, :] = v

    def prep_rest(j):
        zero = zero_s[0]

        def through_xlu(b):
            return jnp.concatenate([pltpu.bitcast(pltpu.roll(pltpu.bitcast(b[:, k:k + 128], i32), zero, 1), bf16)
                                    for k in range(0, CB, 128)], axis=1)
        for _, raw, ext, n, hn in rest:
            for r in range(0, n, RB):
                rows = pl.ds(pl.multiple_of(j * n + r, RB), RB)
                wrows = pl.ds(pl.multiple_of((j * n + r) // 2, RB // 2), RB // 2)
                for c in range(0, hn, CB):
                    e = _right_sums(through_xlu(raw[0, rows, c:c + CB]), raw[0, rows, hn + c:hn + c + CB],
                                    raw[1, rows, c:c + CB], through_xlu(raw[1, rows, hn + c:hn + c + CB]))
                    for i in range(5):
                        ext[i, wrows, c:c + CB] = e[i]

    def qkv_dot(t, op, dst, off):
        ts = _same(t)
        for n, n0 in enumerate(range(0, HD, NB)):
            c = _strassen(lambda i: _dot(load_a(i, ts[n % 4]), pltpu.bitcast(op[i, :, n0:n0 + NB], bf16)))
            for bi, blk in enumerate(c):
                dst[pl.ds(pl.multiple_of(t * M, M) + off + (bi // 2) * HM, HM),
                    (bi % 2) * HD + n0:(bi % 2) * HD + n0 + NB] = blk

    def prologue():
        zero_s[0] = 0
        cp_x(0).start()
        for r in range(QC):
            cp_q(r).start()

        def start_kv(j, carry):
            @pl.when(j < NT - 1)
            def _():
                cp_x(jnp.minimum(j + 1, NT - 1)).start()
            for c in cp_kv(j):
                c.start()
            return carry
        lax.fori_loop(0, NT, start_kv, 0)

        def start_rest(j, carry):
            for c in cp_rest(j):
                c.start()
            return carry
        lax.fori_loop(0, NT, start_rest, 0)
        k_s[pl.ds(0, HALO), :] = jnp.zeros((HALO, D), f32)
        v_s[pl.ds(0, HALO), :] = jnp.zeros((HALO, D), f32)
        cp_x(0).wait()
        layernorm(0)

        def prep_q(r, carry):
            cp_q(r).wait()
            prep_part(0, opq, r, HD // QC)
            return carry
        lax.fori_loop(0, QC, prep_q, 0)

    def q_pass(j, carry):
        nxt = jnp.minimum(j + 1, NT - 1)

        @pl.when(j < NT - 1)
        def _():
            cp_x(nxt).wait()
        for c in cp_kv(j):
            c.wait()
        qkv_dot(j, opq, q_s, 0)
        prep_part(1, opk, j, HD // NT)
        prep_part(2, opv, j, HD // NT)
        layernorm(nxt)
        return carry

    def kv_pass(j, carry):
        for c in cp_rest(j):
            c.wait()
        qkv_dot(j, opk, k_s, HALO)
        qkv_dot(jnp.minimum(j, NT - 1), opv, v_s, HALO)
        prep_rest(j)
        return carry

    def attention(base, r0):
        def taps(ref, m):
            kk = ref[pl.ds(base + r0, R + HALO), m * 128:(m + 1) * 128]
            out = [None] * W
            for r in range(4):
                a = kk[8 - DIL * r:8 - DIL * r + R + 8]
                out[r], out[r + 4] = a[8:R + 8], a[0:R]
            return out
        prods = [[] for _ in range(W)]
        for m in range(8):
            qm = q_s[pl.ds(base + r0, R), m * 128:(m + 1) * 128]
            km = taps(k_s, m)
            for w in range(W):
                prods[w].append(qm * km[w])
        lane = lax.broadcasted_iota(i32, (R, 128), 1)
        pos = base + r0 + lax.broadcasted_iota(i32, (R, 128), 0)
        logits = []
        for w in range(W):
            l = _tree_sum(prods[w])
            l = l + jnp.take_along_axis(l, lane ^ 1, axis=1)
            l = l + jnp.take_along_axis(l, lane ^ 2, axis=1)
            if w > 0:
                l = jnp.where(pos >= DIL * w, l, -1e9)
            logits.append(l)
        mx = functools.reduce(jnp.maximum, logits)
        es = [jnp.exp2((l - mx) * EXP_C) for l in logits]
        inv = 1.0 / _tree_sum(es)
        a = [e * inv for e in es]
        ot = []
        for m in range(8):
            vm = taps(v_s, m)
            ot.append(_tree_sum([a[w] * vm[w] for w in range(W)]))
        o_s[pl.ds(r0, R), :] = jnp.concatenate(_untwist(ot), axis=1)

    def out_copies(t):
        slot = t % 2
        return [pltpu.make_async_copy(
            out_s.at[slot, pl.ds(r0, HM), pl.ds(c0, HD)],
            out_h.at[pl.ds(pl.multiple_of(t * M + r0, HM), HM), pl.ds(c0, HD)], sems.at[SEM_OUT + slot])
            for r0 in (0, HM) for c0 in (0, HD)]

    def ffn_pass(t, carry):
        @pl.when(t >= 2)
        def _():
            for c in out_copies(t - 2):
                c.wait()
        base = pl.multiple_of(t * M, M)
        ts = _same(t)
        g = _combine([_dot(load_a(i, ts[0]), _right(wg_v, wg_e, i, HF, 0, HD, 0, HF)) for i in range(7)])
        u = _combine([_dot(load_a(i, ts[1]), _right(wu_v, wu_e, i, HF, 0, HD, 0, HF)) for i in range(7)])
        e = _left(*[_silu(g[i]) * u[i] for i in range(4)])
        for r0 in range(0, M, R):
            attention(base, r0)
        md = [_dot(e[i], _right(wd_v, wd_e, i, HD, 0, HF, 0, HD)) for i in range(7)]
        gate = [_silu(y) for y in _combine(md)]
        oa = _left(o_s[0:HM, 0:HD], o_s[0:HM, HD:D], o_s[HM:M, 0:HD], o_s[HM:M, HD:D])
        s = _strassen(lambda i: _dot(oa[i], _right(wo_v, wo_e, i, HD, 0, HD, 0, HD)))
        copies = out_copies(t)
        for bi in (2, 1, 0, 3):
            r0, c0 = (bi // 2) * HM, (bi % 2) * HD
            xr = x_s[pl.ds(base + r0, HM), c0:c0 + HD].astype(f32)
            out_s[t % 2, r0:r0 + HM, c0:c0 + HD] = (xr + s[bi] * gate[bi]).astype(bf16)
            copies[bi].start()
        return carry

    prologue()
    lax.fori_loop(0, NT, q_pass, 0)
    lax.fori_loop(0, NT, kv_pass, 0)
    lax.fori_loop(0, NT, ffn_pass, 0)
    for t in (NT - 2, NT - 1):
        for c in out_copies(t):
            c.wait()


@jax.jit
def pallas_recurrent_scan__sliding_local_dilated__swiglu_ffn__prompt_kernel(
    A_x: jax.Array,
    A_wqkv: jax.Array,
    A_wo: jax.Array,
    B_x: jax.Array,
    B_w_gate: jax.Array,
    B_w_up: jax.Array,
    B_w_down: jax.Array,
):
    del B_x
    out = pl.pallas_call(
        _kernel,
        in_specs=[pl.BlockSpec(memory_space=pl.ANY)] * 6,
        out_specs=pl.BlockSpec(memory_space=pl.ANY),
        out_shape=jax.ShapeDtypeStruct((S, D), bf16),
        scratch_shapes=[
            pltpu.VMEM((S, D), bf16),
            pltpu.VMEM((2, HD, 3 * D), bf16), pltpu.VMEM((2, HD, D), bf16),
            pltpu.VMEM((2, HD, F), bf16), pltpu.VMEM((2, HD, F), bf16), pltpu.VMEM((2, HF, D), bf16),
            pltpu.VMEM((7, HD // 2, HD), i32), pltpu.VMEM((7, HD // 2, HD), i32), pltpu.VMEM((7, HD // 2, HD), i32),
            pltpu.VMEM((5, HD // 2, HD), i32),
            pltpu.VMEM((5, HD // 2, HF), i32), pltpu.VMEM((5, HD // 2, HF), i32), pltpu.VMEM((5, HF // 2, HD), i32),
            pltpu.VMEM((7, S // 4, HD), i32),
            pltpu.VMEM((S, D), f32), pltpu.VMEM((S + HALO, D), f32), pltpu.VMEM((S + HALO, D), f32),
            pltpu.VMEM((M, D), f32),
            pltpu.VMEM((2, M, D), bf16),
            pltpu.SMEM((1,), i32),
            pltpu.SemaphoreType.DMA((NSEM,)),
        ],
        compiler_params=pltpu.CompilerParams(
            vmem_limit_bytes=120 * 1024 * 1024, disable_semaphore_checks=True,
            flags={"XLA_TPU_EVENLY_DISTRIBUTE_CRITICAL_NODES": True},
        ),
    )(A_x.reshape(S, D), A_wqkv.reshape(2, HD, 3 * D), A_wo.reshape(2, HD, D), B_w_gate.reshape(2, HD, F),
      B_w_up.reshape(2, HD, F), B_w_down.reshape(2, HF, D))
    return out.reshape(1, S, D)
```

```python
import functools

import jax
from jax import lax
import jax.experimental.pallas as pl
import jax.experimental.pallas.tpu as pltpu
import jax.numpy as jnp
import numpy as np

S, D, F = 2048, 1024, 3584
DH, W, DIL = 32, 8, 2
HALO = 16
HD, HF = D // 2, F // 2
M = 256
HM = M // 2
NT = S // M
R = 16
LG = 16
NB = 128
NO = 512
KVU = 2
QC = 4
RB, CB = 16, 256
EXP_C = float(DH ** -0.5 * np.log2(np.e))
SEM_X, SEM_Q, SEM_KV, SEM_REST, SEM_OUT = 0, NT, NT + QC, 2 * NT + QC, 3 * NT + QC
NSEM = 3 * NT + QC + 2

f32, bf16, i32 = jnp.float32, jnp.bfloat16, jnp.int32


def _twist_level(a, b, bit, lane):
    lo = (lane & (1 << bit)) == 0
    return jnp.where(lo, a, b), jnp.take_along_axis(jnp.where(lo, b, a), lane ^ (1 << bit), axis=1)


def _untwist_level(x, y, bit, lane):
    lo = (lane & (1 << bit)) == 0
    yp = jnp.take_along_axis(y, lane ^ (1 << bit), axis=1)
    return jnp.where(lo, x, yp), jnp.where(lo, yp, x)


def _twist(c):
    lane = lax.broadcasted_iota(i32, c[0].shape, 1)
    n = [None] * 8
    for p in range(4):
        n[p], n[4 + p] = _twist_level(c[2 * p], c[2 * p + 1], 4, lane)
    c, n = n, [None] * 8
    for g in range(0, 8, 4):
        for p in range(2):
            n[g + p], n[g + 2 + p] = _twist_level(c[g + 2 * p], c[g + 2 * p + 1], 3, lane)
    c, n = n, [None] * 8
    for g in range(0, 8, 2):
        n[g], n[g + 1] = _twist_level(c[g], c[g + 1], 2, lane)
    return n


def _untwist(c):
    lane = lax.broadcasted_iota(i32, c[0].shape, 1)
    n = [None] * 8
    for g in range(0, 8, 2):
        n[g], n[g + 1] = _untwist_level(c[g], c[g + 1], 2, lane)
    c, n = n, [None] * 8
    for g in range(0, 8, 4):
        for p in range(2):
            n[g + 2 * p], n[g + 2 * p + 1] = _untwist_level(c[g + p], c[g + 2 + p], 3, lane)
    c, n = n, [None] * 8
    for p in range(4):
        n[2 * p], n[2 * p + 1] = _untwist_level(c[p], c[4 + p], 4, lane)
    return n


def _dot(a, b):
    return jnp.dot(a, b, preferred_element_type=f32)


def _left_f32(a11, a12, a21, a22):
    return [a11 + a22, a21 + a22, a11, a22, a11 + a12, a21 - a11, a12 - a22]


def _left(*blocks):
    return [a.astype(bf16) for a in _left_f32(*blocks)]


def _right_sums(b11, b12, b21, b22):
    b11, b12, b21, b22 = [b.astype(f32) for b in (b11, b12, b21, b22)]
    return [pltpu.bitcast(v.astype(bf16), i32) for v in (b11 + b22, b12 - b22, b21 - b11, b11 + b12, b21 + b22)]


def _right(raw, ext, i, hn, k0, kn, n0, nn):
    if i in (1, 4):
        r = 0 if i == 1 else 1
        return raw[r, k0:k0 + kn, r * hn + n0:r * hn + n0 + nn]
    e = {0: 0, 2: 1, 3: 2, 5: 3, 6: 4}[i]
    return pltpu.bitcast(ext[e, k0 // 2:(k0 + kn) // 2, n0:n0 + nn], bf16)


def _strassen(prod):
    m2, m4 = prod(1), prod(3)
    c21 = m2 + m4
    m3 = prod(2)
    c22 = m3 - m2
    m5 = prod(4)
    c12 = m3 + m5
    c11 = m4 - m5
    m1 = prod(0)
    c11 = c11 + m1 + prod(6)
    c22 = c22 + m1 + prod(5)
    return c11, c12, c21, c22


def _combine(m):
    return m[0] + m[3] - m[4] + m[6], m[2] + m[4], m[1] + m[3], m[0] - m[1] + m[2] + m[5]


def _tree_sum(xs):
    xs = list(xs)
    while len(xs) > 1:
        xs = [xs[i] + xs[i + 1] for i in range(0, len(xs), 2)]
    return xs[0]


def _silu(g):
    hg = 0.5 * g
    return hg * jnp.tanh(hg) + hg


def _ds(i, n):
    return pl.ds(pl.multiple_of(i * n, n), n)


def _same(t):
    return t, jnp.minimum(t, NT - 1), jnp.maximum(t, 0), jnp.clip(t, 0, NT)


def _kernel(x_h, wqkv_h, wo_h, wg_h, wu_h, wd_h, out_h,
            x_s, wqkv_v, wo_v, wg_v, wu_v, wd_v, opq, opk, opv, wo_e, wg_e, wu_e, wd_e,
            xa_s, q_s, k_s, v_s, o_s, out_s, zero_s, sems):

    def cp_x(t):
        return pltpu.make_async_copy(x_h.at[_ds(t, M), :], x_s.at[_ds(t, M), :], sems.at[SEM_X + t])

    def cp_w(p, rows, sem):
        return pltpu.make_async_copy(wqkv_h.at[:, rows, pl.ds(p * D, D)], wqkv_v.at[:, rows, pl.ds(p * D, D)],
                                     sems.at[sem])

    def cp_q(r):
        return cp_w(0, _ds(r, HD // QC), SEM_Q + r)

    def cp_kv(j):
        return [cp_w(p, _ds(j, HD // NT), SEM_KV + j) for p in (1, 2)]

    rest = [(wg_h, wg_v, wg_e, HD // NT, HF), (wu_h, wu_v, wu_e, HD // NT, HF),
            (wd_h, wd_v, wd_e, HF // NT, HD), (wo_h, wo_v, wo_e, HD // NT, HD)]

    def cp_rest(j):
        return [pltpu.make_async_copy(src.at[:, _ds(j, n), :], raw.at[:, _ds(j, n), :], sems.at[SEM_REST + j])
                for src, raw, _, n, _ in rest]

    def layernorm(t):
        def norm(r0):
            x = x_s[pl.ds(pl.multiple_of(t * M + r0, LG), LG), :].astype(f32)
            xc = x - jnp.mean(x, axis=-1, keepdims=True)
            return xc * lax.rsqrt(jnp.mean(xc * xc, axis=-1, keepdims=True) + 1e-5)
        for r in range(0, HM, LG):
            top, bot = norm(r), norm(HM + r)
            a = _left(top[:, :HD], top[:, HD:], bot[:, :HD], bot[:, HD:])
            for i in range(7):
                xa_s[i, pl.ds(pl.multiple_of(t * (HM // 2) + r // 2, LG // 2), LG // 2), :] = pltpu.bitcast(a[i], i32)

    def load_a(i, t):
        return pltpu.bitcast(xa_s[i, _ds(t, HM // 2), :], bf16)

    def prep_part(p, op, r, n):
        rows, wrows = _ds(r, n), _ds(r, n // 2)
        blk = []
        for half in range(2):
            w = pltpu.bitcast(wqkv_v[half, rows, pl.ds(p * D, D)], i32)
            t = _twist([w[:, c * 128:(c + 1) * 128] for c in range(8)])
            blk += [jnp.concatenate(t[:4], axis=1), jnp.concatenate(t[4:], axis=1)]
        sums = _right_sums(*[pltpu.bitcast(b, bf16) for b in blk])
        for i, v in zip((0, 2, 3, 5, 6, 1, 4), sums + [blk[0], blk[3]]):
            op[i, wrows, :] = v

    def prep_rest(j):
        zero = zero_s[0]

        def through_xlu(b):
            return jnp.concatenate([pltpu.bitcast(pltpu.roll(pltpu.bitcast(b[:, k:k + 128], i32), zero, 1), bf16)
                                    for k in range(0, CB, 128)], axis=1)
        for _, raw, ext, n, hn in rest:
            for r in range(0, n, RB):
                rows = pl.ds(pl.multiple_of(j * n + r, RB), RB)
                wrows = pl.ds(pl.multiple_of((j * n + r) // 2, RB // 2), RB // 2)
                for c in range(0, hn, CB):
                    e = _right_sums(through_xlu(raw[0, rows, c:c + CB]), raw[0, rows, hn + c:hn + c + CB],
                                    raw[1, rows, c:c + CB], through_xlu(raw[1, rows, hn + c:hn + c + CB]))
                    for i in range(5):
                        ext[i, wrows, c:c + CB] = e[i]

    def qkv_dot(t, op, dst, off):
        ts = _same(t)
        for n, n0 in enumerate(range(0, HD, NB)):
            c = _strassen(lambda i: _dot(load_a(i, ts[n % 4]), pltpu.bitcast(op[i, :, n0:n0 + NB], bf16)))
            for bi, blk in enumerate(c):
                dst[pl.ds(pl.multiple_of(t * M, M) + off + (bi // 2) * HM, HM),
                    (bi % 2) * HD + n0:(bi % 2) * HD + n0 + NB] = blk

    def prologue():
        zero_s[0] = 0
        cp_x(0).start()
        for r in range(QC):
            cp_q(r).start()

        def start_kv(j, carry):
            @pl.when(j < NT - 1)
            def _():
                cp_x(jnp.minimum(j + 1, NT - 1)).start()
            for c in cp_kv(j):
                c.start()
            return carry
        lax.fori_loop(0, NT, start_kv, 0)

        def start_rest(j, carry):
            for c in cp_rest(j):
                c.start()
            return carry
        lax.fori_loop(0, NT, start_rest, 0)
        k_s[pl.ds(0, HALO), :] = jnp.zeros((HALO, D), f32)
        v_s[pl.ds(0, HALO), :] = jnp.zeros((HALO, D), f32)
        cp_x(0).wait()
        layernorm(0)

        def prep_q(r, carry):
            cp_q(r).wait()
            prep_part(0, opq, r, HD // QC)
            return carry
        lax.fori_loop(0, QC, prep_q, 0)

    def q_pass(j, carry):
        nxt = jnp.minimum(j + 1, NT - 1)

        @pl.when(j < NT - 1)
        def _():
            cp_x(nxt).wait()
        for c in cp_kv(j):
            c.wait()
        qkv_dot(j, opq, q_s, 0)
        prep_part(1, opk, j, HD // NT)
        prep_part(2, opv, j, HD // NT)
        layernorm(nxt)
        return carry

    def kv_pass(i, carry):
        for u in range(KVU):
            for c in cp_rest(KVU * i + u):
                c.wait()
        for u in range(KVU):
            j = KVU * i + u
            qkv_dot(j, opk, k_s, HALO)
            qkv_dot(jnp.minimum(j, NT - 1), opv, v_s, HALO)
            prep_rest(j)
        return carry

    def attention(base, r0):
        def taps(ref, m):
            kk = ref[pl.ds(base + r0, R + HALO), m * 128:(m + 1) * 128]
            out = [None] * W
            for r in range(4):
                a = kk[8 - DIL * r:8 - DIL * r + R + 8]
                out[r], out[r + 4] = a[8:R + 8], a[0:R]
            return out
        prods = [[] for _ in range(W)]
        for m in range(8):
            qm = q_s[pl.ds(base + r0, R), m * 128:(m + 1) * 128]
            km = taps(k_s, m)
            for w in range(W):
                prods[w].append(qm * km[w])
        lane = lax.broadcasted_iota(i32, (R, 128), 1)
        pos = base + r0 + lax.broadcasted_iota(i32, (R, 128), 0)
        logits = []
        for w in range(W):
            l = _tree_sum(prods[w])
            l = l + jnp.take_along_axis(l, lane ^ 1, axis=1)
            l = l + jnp.take_along_axis(l, lane ^ 2, axis=1)
            if w > 0:
                l = jnp.where(pos >= DIL * w, l, -1e9)
            logits.append(l)
        mx = functools.reduce(jnp.maximum, logits)
        es = [jnp.exp2((l - mx) * EXP_C) for l in logits]
        inv = 1.0 / _tree_sum(es)
        a = [e * inv for e in es]
        ot = []
        for m in range(8):
            vm = taps(v_s, m)
            ot.append(_tree_sum([a[w] * vm[w] for w in range(W)]))
        o_s[pl.ds(r0, R), :] = jnp.concatenate(_untwist(ot), axis=1)

    def out_copies(t):
        slot = t % 2
        return [pltpu.make_async_copy(
            out_s.at[slot, pl.ds(r0, HM), pl.ds(c0, HD)],
            out_h.at[pl.ds(pl.multiple_of(t * M + r0, HM), HM), pl.ds(c0, HD)], sems.at[SEM_OUT + slot])
            for r0 in (0, HM) for c0 in (0, HD)]

    def ffn_pass(t, carry):
        @pl.when(t >= 2)
        def _():
            for c in out_copies(t - 2):
                c.wait()
        base = pl.multiple_of(t * M, M)
        ts = _same(t)
        g = _combine([_dot(load_a(i, ts[0]), _right(wg_v, wg_e, i, HF, 0, HD, 0, HF)) for i in range(7)])
        u = _combine([_dot(load_a(i, ts[1]), _right(wu_v, wu_e, i, HF, 0, HD, 0, HF)) for i in range(7)])
        e = _left(*[_silu(g[i]) * u[i] for i in range(4)])
        for r0 in range(0, M, R):
            attention(base, r0)
        md = [_dot(e[i], _right(wd_v, wd_e, i, HD, 0, HF, 0, HD)) for i in range(7)]
        gate = [_silu(y) for y in _combine(md)]
        oa = _left(o_s[0:HM, 0:HD], o_s[0:HM, HD:D], o_s[HM:M, 0:HD], o_s[HM:M, HD:D])
        s = _strassen(lambda i: _dot(oa[i], _right(wo_v, wo_e, i, HD, 0, HD, 0, HD)))
        copies = out_copies(t)
        for bi in (2, 1, 0, 3):
            r0, c0 = (bi // 2) * HM, (bi % 2) * HD
            xr = x_s[pl.ds(base + r0, HM), c0:c0 + HD].astype(f32)
            out_s[t % 2, r0:r0 + HM, c0:c0 + HD] = (xr + s[bi] * gate[bi]).astype(bf16)
            copies[bi].start()
        return carry

    prologue()
    lax.fori_loop(0, NT, q_pass, 0)
    lax.fori_loop(0, NT // KVU, kv_pass, 0)
    lax.fori_loop(0, NT, ffn_pass, 0)
    for t in (NT - 2, NT - 1):
        for c in out_copies(t):
            c.wait()


@jax.jit
def pallas_recurrent_scan__sliding_local_dilated__swiglu_ffn__prompt_kernel(
    A_x: jax.Array,
    A_wqkv: jax.Array,
    A_wo: jax.Array,
    B_x: jax.Array,
    B_w_gate: jax.Array,
    B_w_up: jax.Array,
    B_w_down: jax.Array,
):
    del B_x
    out = pl.pallas_call(
        _kernel,
        in_specs=[pl.BlockSpec(memory_space=pl.ANY)] * 6,
        out_specs=pl.BlockSpec(memory_space=pl.ANY),
        out_shape=jax.ShapeDtypeStruct((S, D), bf16),
        scratch_shapes=[
            pltpu.VMEM((S, D), bf16),
            pltpu.VMEM((2, HD, 3 * D), bf16), pltpu.VMEM((2, HD, D), bf16),
            pltpu.VMEM((2, HD, F), bf16), pltpu.VMEM((2, HD, F), bf16), pltpu.VMEM((2, HF, D), bf16),
            pltpu.VMEM((7, HD // 2, HD), i32), pltpu.VMEM((7, HD // 2, HD), i32), pltpu.VMEM((7, HD // 2, HD), i32),
            pltpu.VMEM((5, HD // 2, HD), i32),
            pltpu.VMEM((5, HD // 2, HF), i32), pltpu.VMEM((5, HD // 2, HF), i32), pltpu.VMEM((5, HF // 2, HD), i32),
            pltpu.VMEM((7, S // 4, HD), i32),
            pltpu.VMEM((S, D), f32), pltpu.VMEM((S + HALO, D), f32), pltpu.VMEM((S + HALO, D), f32),
            pltpu.VMEM((M, D), f32),
            pltpu.VMEM((2, M, D), bf16),
            pltpu.SMEM((1,), i32),
            pltpu.SemaphoreType.DMA((NSEM,)),
        ],
        compiler_params=pltpu.CompilerParams(
            vmem_limit_bytes=120 * 1024 * 1024, disable_semaphore_checks=True,
            flags={"XLA_TPU_EVENLY_DISTRIBUTE_CRITICAL_NODES": True},
        ),
    )(A_x.reshape(S, D), A_wqkv.reshape(2, HD, 3 * D), A_wo.reshape(2, HD, D), B_w_gate.reshape(2, HD, F),
      B_w_up.reshape(2, HD, F), B_w_down.reshape(2, HF, D))
    return out.reshape(1, S, D)
```

```python
import functools

import jax
from jax import lax
import jax.experimental.pallas as pl
import jax.experimental.pallas.tpu as pltpu
import jax.numpy as jnp
import numpy as np

S, D, F = 2048, 1024, 3584
DH, W, DIL = 32, 8, 2
HALO = 16
HD, HF = D // 2, F // 2
M = 256
HM = M // 2
NT = S // M
R = 16
LG = 16
NB = 128
KVU = 2
QC = 4
RB, CB = 16, 256
EXP_C = float(DH ** -0.5 * np.log2(np.e))
MASKED = float(-1e9 * DH ** 0.5)
SEM_X, SEM_Q, SEM_KV, SEM_REST, SEM_OUT = 0, NT, NT + QC, 2 * NT + QC, 3 * NT + QC
NSEM = 3 * NT + QC + 2

f32, bf16, i32 = jnp.float32, jnp.bfloat16, jnp.int32


def _twist_level(a, b, bit, lane):
    lo = (lane & (1 << bit)) == 0
    return jnp.where(lo, a, b), jnp.take_along_axis(jnp.where(lo, b, a), lane ^ (1 << bit), axis=1)


def _untwist_level(x, y, bit, lane):
    lo = (lane & (1 << bit)) == 0
    yp = jnp.take_along_axis(y, lane ^ (1 << bit), axis=1)
    return jnp.where(lo, x, yp), jnp.where(lo, yp, x)


def _twist(c):
    lane = lax.broadcasted_iota(i32, c[0].shape, 1)
    n = [None] * 8
    for p in range(4):
        n[p], n[4 + p] = _twist_level(c[2 * p], c[2 * p + 1], 4, lane)
    c, n = n, [None] * 8
    for g in range(0, 8, 4):
        for p in range(2):
            n[g + p], n[g + 2 + p] = _twist_level(c[g + 2 * p], c[g + 2 * p + 1], 3, lane)
    c, n = n, [None] * 8
    for g in range(0, 8, 2):
        n[g], n[g + 1] = _twist_level(c[g], c[g + 1], 2, lane)
    return n


def _untwist(c):
    lane = lax.broadcasted_iota(i32, c[0].shape, 1)
    n = [None] * 8
    for g in range(0, 8, 2):
        n[g], n[g + 1] = _untwist_level(c[g], c[g + 1], 2, lane)
    c, n = n, [None] * 8
    for g in range(0, 8, 4):
        for p in range(2):
            n[g + 2 * p], n[g + 2 * p + 1] = _untwist_level(c[g + p], c[g + 2 + p], 3, lane)
    c, n = n, [None] * 8
    for p in range(4):
        n[2 * p], n[2 * p + 1] = _untwist_level(c[p], c[4 + p], 4, lane)
    return n


def _dot(a, b):
    return jnp.dot(a, b, preferred_element_type=f32)


def _left_f32(a11, a12, a21, a22):
    return [a11 + a22, a21 + a22, a11, a22, a11 + a12, a21 - a11, a12 - a22]


def _left(*blocks):
    return [a.astype(bf16) for a in _left_f32(*blocks)]


def _right_sums(b11, b12, b21, b22):
    b11, b12, b21, b22 = [b.astype(f32) for b in (b11, b12, b21, b22)]
    return [pltpu.bitcast(v.astype(bf16), i32) for v in (b11 + b22, b12 - b22, b21 - b11, b11 + b12, b21 + b22)]


def _right(raw, ext, i, hn, k0, kn, n0, nn):
    if i in (1, 4):
        r = 0 if i == 1 else 1
        return raw[r, k0:k0 + kn, r * hn + n0:r * hn + n0 + nn]
    e = {0: 0, 2: 1, 3: 2, 5: 3, 6: 4}[i]
    return pltpu.bitcast(ext[e, k0 // 2:(k0 + kn) // 2, n0:n0 + nn], bf16)


def _strassen(prod):
    m2, m4 = prod(1), prod(3)
    c21 = m2 + m4
    m3 = prod(2)
    c22 = m3 - m2
    m5 = prod(4)
    c12 = m3 + m5
    c11 = m4 - m5
    m1 = prod(0)
    c11 = c11 + m1 + prod(6)
    c22 = c22 + m1 + prod(5)
    return c11, c12, c21, c22


def _combine(m):
    return m[0] + m[3] - m[4] + m[6], m[2] + m[4], m[1] + m[3], m[0] - m[1] + m[2] + m[5]


def _tree_sum(xs):
    xs = list(xs)
    while len(xs) > 1:
        xs = [xs[i] + xs[i + 1] for i in range(0, len(xs), 2)]
    return xs[0]


def _silu(g):
    hg = 0.5 * g
    return hg * jnp.tanh(hg) + hg


def _ds(i, n):
    return pl.ds(pl.multiple_of(i * n, n), n)


def _same(t):
    return t, jnp.minimum(t, NT - 1), jnp.maximum(t, 0), jnp.clip(t, 0, NT)


def _kernel(x_h, wqkv_h, wo_h, wg_h, wu_h, wd_h, out_h,
            x_s, wqkv_v, wo_v, wg_v, wu_v, wd_v, opq, opk, opv, wo_e, wg_e, wu_e, wd_e,
            xa_s, q_s, k_s, v_s, o_s, out_s, zero_s, sems):

    def cp_x(t):
        return pltpu.make_async_copy(x_h.at[_ds(t, M), :], x_s.at[_ds(t, M), :], sems.at[SEM_X + t])

    def cp_w(p, rows, sem):
        return pltpu.make_async_copy(wqkv_h.at[:, rows, pl.ds(p * D, D)], wqkv_v.at[:, rows, pl.ds(p * D, D)],
                                     sems.at[sem])

    def cp_q(r):
        return cp_w(0, _ds(r, HD // QC), SEM_Q + r)

    def cp_kv(j):
        return [cp_w(p, _ds(j, HD // NT), SEM_KV + j) for p in (1, 2)]

    rest = [(wg_h, wg_v, wg_e, HD // NT, HF), (wu_h, wu_v, wu_e, HD // NT, HF),
            (wd_h, wd_v, wd_e, HF // NT, HD), (wo_h, wo_v, wo_e, HD // NT, HD)]

    def cp_rest(j):
        return [pltpu.make_async_copy(src.at[:, _ds(j, n), :], raw.at[:, _ds(j, n), :], sems.at[SEM_REST + j])
                for src, raw, _, n, _ in rest]

    def layernorm(t):
        def norm(r0):
            x = x_s[pl.ds(pl.multiple_of(t * M + r0, LG), LG), :].astype(f32)
            xc = x - jnp.mean(x, axis=-1, keepdims=True)
            return xc * lax.rsqrt(jnp.mean(xc * xc, axis=-1, keepdims=True) + 1e-5)
        for r in range(0, HM, LG):
            top, bot = norm(r), norm(HM + r)
            a = _left(top[:, :HD], top[:, HD:], bot[:, :HD], bot[:, HD:])
            for i in range(7):
                xa_s[i, pl.ds(pl.multiple_of(t * (HM // 2) + r // 2, LG // 2), LG // 2), :] = pltpu.bitcast(a[i], i32)

    def load_a(i, t):
        return pltpu.bitcast(xa_s[i, _ds(t, HM // 2), :], bf16)

    def prep_part(p, op, r, n):
        rows, wrows = _ds(r, n), _ds(r, n // 2)
        blk = []
        for half in range(2):
            w = pltpu.bitcast(wqkv_v[half, rows, pl.ds(p * D, D)], i32)
            t = _twist([w[:, c * 128:(c + 1) * 128] for c in range(8)])
            blk += [jnp.concatenate(t[:4], axis=1), jnp.concatenate(t[4:], axis=1)]
        sums = _right_sums(*[pltpu.bitcast(b, bf16) for b in blk])
        for i, v in zip((0, 2, 3, 5, 6, 1, 4), sums + [blk[0], blk[3]]):
            op[i, wrows, :] = v

    def prep_rest(j):
        zero = zero_s[0]

        def through_xlu(b):
            return jnp.concatenate([pltpu.bitcast(pltpu.roll(pltpu.bitcast(b[:, k:k + 128], i32), zero, 1), bf16)
                                    for k in range(0, CB, 128)], axis=1)
        for _, raw, ext, n, hn in rest:
            for r in range(0, n, RB):
                rows = pl.ds(pl.multiple_of(j * n + r, RB), RB)
                wrows = pl.ds(pl.multiple_of((j * n + r) // 2, RB // 2), RB // 2)
                for c in range(0, hn, CB):
                    e = _right_sums(through_xlu(raw[0, rows, c:c + CB]), raw[0, rows, hn + c:hn + c + CB],
                                    raw[1, rows, c:c + CB], through_xlu(raw[1, rows, hn + c:hn + c + CB]))
                    for i in range(5):
                        ext[i, wrows, c:c + CB] = e[i]

    def qkv_dot(t, op, dst, off):
        ts = _same(t)
        for n, n0 in enumerate(range(0, HD, NB)):
            c = _strassen(lambda i: _dot(load_a(i, ts[n % 4]), pltpu.bitcast(op[i, :, n0:n0 + NB], bf16)))
            for bi, blk in enumerate(c):
                dst[pl.ds(pl.multiple_of(t * M, M) + off + (bi // 2) * HM, HM),
                    (bi % 2) * HD + n0:(bi % 2) * HD + n0 + NB] = blk

    def prologue():
        zero_s[0] = 0
        cp_x(0).start()
        for r in range(QC):
            cp_q(r).start()

        def start_kv(j, carry):
            @pl.when(j < NT - 1)
            def _():
                cp_x(jnp.minimum(j + 1, NT - 1)).start()
            for c in cp_kv(j):
                c.start()
            return carry
        lax.fori_loop(0, NT, start_kv, 0)

        def start_rest(j, carry):
            for c in cp_rest(j):
                c.start()
            return carry
        lax.fori_loop(0, NT, start_rest, 0)
        k_s[pl.ds(0, HALO), :] = jnp.zeros((HALO, D), f32)
        cp_x(0).wait()
        layernorm(0)

        def prep_q(r, carry):
            cp_q(r).wait()
            prep_part(0, opq, r, HD // QC)
            return carry
        lax.fori_loop(0, QC, prep_q, 0)

    def q_pass(j, carry):
        nxt = jnp.minimum(j + 1, NT - 1)

        @pl.when(j < NT - 1)
        def _():
            cp_x(nxt).wait()
        for c in cp_kv(j):
            c.wait()
        qkv_dot(j, opq, q_s, 0)
        prep_part(1, opk, j, HD // NT)
        prep_part(2, opv, j, HD // NT)
        layernorm(nxt)
        return carry

    def kv_pass(i, carry):
        for u in range(KVU):
            for c in cp_rest(KVU * i + u):
                c.wait()
        for u in range(KVU):
            j = KVU * i + u
            qkv_dot(j, opk, k_s, HALO)
            qkv_dot(jnp.minimum(j, NT - 1), opv, v_s, HALO)
            prep_rest(j)
        return carry

    def attention(base, r0):
        def taps(ref, m):
            kk = ref[pl.ds(base + r0, R + HALO), m * 128:(m + 1) * 128]
            out = [None] * W
            for r in range(4):
                a = kk[8 - DIL * r:8 - DIL * r + R + 8]
                out[r], out[r + 4] = a[8:R + 8], a[0:R]
            return out
        prods = [[] for _ in range(W)]
        for m in range(8):
            qm = q_s[pl.ds(base + r0, R), m * 128:(m + 1) * 128]
            km = taps(k_s, m)
            for w in range(W):
                prods[w].append(qm * km[w])
        lane = lax.broadcasted_iota(i32, (R, 128), 1)
        pos = base + r0 + lax.broadcasted_iota(i32, (R, 128), 0)
        logits = []
        for w in range(W):
            l = _tree_sum(prods[w])
            l = l + jnp.take_along_axis(l, lane ^ 1, axis=1)
            l = l + jnp.take_along_axis(l, lane ^ 2, axis=1)
            if w > 0:
                l = jnp.where(pos >= DIL * w, l, MASKED)
            logits.append(l)
        mx = functools.reduce(jnp.maximum, logits)
        es = [jnp.exp2((l - mx) * EXP_C) for l in logits]
        inv = 1.0 / _tree_sum(es)
        a = [e * inv for e in es]
        ot = []
        for m in range(8):
            vm = taps(v_s, m)
            ot.append(_tree_sum([a[w] * vm[w] for w in range(W)]))
        o_s[pl.ds(r0, R), :] = jnp.concatenate(_untwist(ot), axis=1)

    def out_copies(t):
        slot = t % 2
        return [pltpu.make_async_copy(
            out_s.at[slot, pl.ds(r0, HM), pl.ds(c0, HD)],
            out_h.at[pl.ds(pl.multiple_of(t * M + r0, HM), HM), pl.ds(c0, HD)], sems.at[SEM_OUT + slot])
            for r0 in (0, HM) for c0 in (0, HD)]

    def ffn_pass(t, carry):
        @pl.when(t >= 2)
        def _():
            for c in out_copies(t - 2):
                c.wait()
        base = pl.multiple_of(t * M, M)
        ts = _same(t)
        g = _combine([_dot(load_a(i, ts[0]), _right(wg_v, wg_e, i, HF, 0, HD, 0, HF)) for i in range(7)])
        u = _combine([_dot(load_a(i, ts[1]), _right(wu_v, wu_e, i, HF, 0, HD, 0, HF)) for i in range(7)])
        e = _left(*[_silu(g[i]) * u[i] for i in range(4)])
        for r0 in range(0, M, R):
            attention(base, r0)
        md = [_dot(e[i], _right(wd_v, wd_e, i, HD, 0, HF, 0, HD)) for i in range(7)]
        gate = [_silu(y) for y in _combine(md)]
        oa = _left(o_s[0:HM, 0:HD], o_s[0:HM, HD:D], o_s[HM:M, 0:HD], o_s[HM:M, HD:D])
        s = _strassen(lambda i: _dot(oa[i], _right(wo_v, wo_e, i, HD, 0, HD, 0, HD)))
        copies = out_copies(t)
        for bi in (2, 1, 0, 3):
            r0, c0 = (bi // 2) * HM, (bi % 2) * HD
            xr = x_s[pl.ds(base + r0, HM), c0:c0 + HD].astype(f32)
            out_s[t % 2, r0:r0 + HM, c0:c0 + HD] = (xr + s[bi] * gate[bi]).astype(bf16)
            copies[bi].start()
        return carry

    prologue()
    lax.fori_loop(0, NT, q_pass, 0)
    lax.fori_loop(0, NT // KVU, kv_pass, 0)
    v_s[pl.ds(0, HALO), :] = jnp.broadcast_to(v_s[pl.ds(HALO, 1), :], (HALO, D))
    lax.fori_loop(0, NT, ffn_pass, 0)
    for t in (NT - 2, NT - 1):
        for c in out_copies(t):
            c.wait()


@jax.jit
def pallas_recurrent_scan__sliding_local_dilated__swiglu_ffn__prompt_kernel(
    A_x: jax.Array,
    A_wqkv: jax.Array,
    A_wo: jax.Array,
    B_x: jax.Array,
    B_w_gate: jax.Array,
    B_w_up: jax.Array,
    B_w_down: jax.Array,
):
    del B_x
    out = pl.pallas_call(
        _kernel,
        in_specs=[pl.BlockSpec(memory_space=pl.ANY)] * 6,
        out_specs=pl.BlockSpec(memory_space=pl.ANY),
        out_shape=jax.ShapeDtypeStruct((S, D), bf16),
        scratch_shapes=[
            pltpu.VMEM((S, D), bf16),
            pltpu.VMEM((2, HD, 3 * D), bf16), pltpu.VMEM((2, HD, D), bf16),
            pltpu.VMEM((2, HD, F), bf16), pltpu.VMEM((2, HD, F), bf16), pltpu.VMEM((2, HF, D), bf16),
            pltpu.VMEM((7, HD // 2, HD), i32), pltpu.VMEM((7, HD // 2, HD), i32), pltpu.VMEM((7, HD // 2, HD), i32),
            pltpu.VMEM((5, HD // 2, HD), i32),
            pltpu.VMEM((5, HD // 2, HF), i32), pltpu.VMEM((5, HD // 2, HF), i32), pltpu.VMEM((5, HF // 2, HD), i32),
            pltpu.VMEM((7, S // 4, HD), i32),
            pltpu.VMEM((S, D), f32), pltpu.VMEM((S + HALO, D), f32), pltpu.VMEM((S + HALO, D), f32),
            pltpu.VMEM((M, D), f32),
            pltpu.VMEM((2, M, D), bf16),
            pltpu.SMEM((1,), i32),
            pltpu.SemaphoreType.DMA((NSEM,)),
        ],
        compiler_params=pltpu.CompilerParams(
            vmem_limit_bytes=120 * 1024 * 1024,
            disable_semaphore_checks=True,
            flags={"XLA_TPU_EVENLY_DISTRIBUTE_CRITICAL_NODES": True},
        ),
    )(A_x.reshape(S, D), A_wqkv.reshape(2, HD, 3 * D), A_wo.reshape(2, HD, D), B_w_gate.reshape(2, HD, F),
      B_w_up.reshape(2, HD, F), B_w_down.reshape(2, HF, D))
    return out.reshape(1, S, D)
```

```python
import functools

import jax
from jax import lax
import jax.experimental.pallas as pl
import jax.experimental.pallas.tpu as pltpu
import jax.numpy as jnp
import numpy as np

S, D, F = 2048, 1024, 3584
DH, W, DIL = 32, 8, 2
HALO = 16
HD, HF, QD, QF = D // 2, F // 2, D // 4, F // 4
M = 256
HM = M // 2
NT = S // M
R = 16
LG = 16
NB = 128
FCHUNKS = ((0, 384), (384, 512))
KVU = 2
QC = 4
RB, CB = 16, 256
EXP_C = float(DH ** -0.5 * np.log2(np.e))
MASKED = float(-1e9 * DH ** 0.5)
SEM_X, SEM_Q, SEM_KV, SEM_REST, SEM_OUT = 0, NT, NT + QC, 2 * NT + QC, 3 * NT + QC
NSEM = 3 * NT + QC + 2

f32, bf16, i32 = jnp.float32, jnp.bfloat16, jnp.int32


def _twist_level(a, b, bit, lane):
    lo = (lane & (1 << bit)) == 0
    return jnp.where(lo, a, b), jnp.take_along_axis(jnp.where(lo, b, a), lane ^ (1 << bit), axis=1)


def _untwist_level(x, y, bit, lane):
    lo = (lane & (1 << bit)) == 0
    yp = jnp.take_along_axis(y, lane ^ (1 << bit), axis=1)
    return jnp.where(lo, x, yp), jnp.where(lo, yp, x)


def _twist(c):
    lane = lax.broadcasted_iota(i32, c[0].shape, 1)
    n = [None] * 8
    for p in range(4):
        n[p], n[4 + p] = _twist_level(c[2 * p], c[2 * p + 1], 4, lane)
    c, n = n, [None] * 8
    for g in range(0, 8, 4):
        for p in range(2):
            n[g + p], n[g + 2 + p] = _twist_level(c[g + 2 * p], c[g + 2 * p + 1], 3, lane)
    c, n = n, [None] * 8
    for g in range(0, 8, 2):
        n[g], n[g + 1] = _twist_level(c[g], c[g + 1], 2, lane)
    return n


def _untwist(c):
    lane = lax.broadcasted_iota(i32, c[0].shape, 1)
    n = [None] * 8
    for g in range(0, 8, 2):
        n[g], n[g + 1] = _untwist_level(c[g], c[g + 1], 2, lane)
    c, n = n, [None] * 8
    for g in range(0, 8, 4):
        for p in range(2):
            n[g + 2 * p], n[g + 2 * p + 1] = _untwist_level(c[g + p], c[g + 2 + p], 3, lane)
    c, n = n, [None] * 8
    for p in range(4):
        n[2 * p], n[2 * p + 1] = _untwist_level(c[p], c[4 + p], 4, lane)
    return n


def _dot(a, b):
    return jnp.dot(a, b, preferred_element_type=f32)


def _left_f32(a11, a12, a21, a22):
    return [a11 + a22, a21 + a22, a11, a22, a11 + a12, a21 - a11, a12 - a22]


def _left(*blocks):
    return [a.astype(bf16) for a in _left_f32(*blocks)]


def _right_sums(b11, b12, b21, b22):
    b11, b12, b21, b22 = [b.astype(f32) for b in (b11, b12, b21, b22)]
    return [pltpu.bitcast(v.astype(bf16), i32) for v in (b11 + b22, b12 - b22, b21 - b11, b11 + b12, b21 + b22)]


def _right_f32(b11, b12, b21, b22):
    return [b11 + b22, b11, b12 - b22, b21 - b11, b22, b11 + b12, b21 + b22]


RAW2 = {(1, 1): (0, 0), (1, 4): (1, 1), (4, 1): (2, 2), (4, 4): (3, 3)}
SLOT2 = {p: n for n, p in enumerate(p for p in ((i, k) for i in range(7) for k in range(7)) if p not in RAW2)}


def _right(raw, ext, i, hn, k0, kn, n0, nn):
    if i in (1, 4):
        r = 0 if i == 1 else 1
        return raw[r, k0:k0 + kn, r * hn + n0:r * hn + n0 + nn]
    e = {0: 0, 2: 1, 3: 2, 5: 3, 6: 4}[i]
    return pltpu.bitcast(ext[e, k0 // 2:(k0 + kn) // 2, n0:n0 + nn], bf16)


def _strassen(prod):
    m2, m4 = prod(1), prod(3)
    c21 = m2 + m4
    m3 = prod(2)
    c22 = m3 - m2
    m5 = prod(4)
    c12 = m3 + m5
    c11 = m4 - m5
    m1 = prod(0)
    c11 = c11 + m1 + prod(6)
    c22 = c22 + m1 + prod(5)
    return c11, c12, c21, c22


def _combine(m):
    return m[0] + m[3] - m[4] + m[6], m[2] + m[4], m[1] + m[3], m[0] - m[1] + m[2] + m[5]


def _tree_sum(xs):
    xs = list(xs)
    while len(xs) > 1:
        xs = [xs[i] + xs[i + 1] for i in range(0, len(xs), 2)]
    return xs[0]


def _silu(g):
    hg = 0.5 * g
    return hg * jnp.tanh(hg) + hg


def _ds(i, n):
    return pl.ds(pl.multiple_of(i * n, n), n)


def _same(t):
    return t, jnp.minimum(t, NT - 1), jnp.maximum(t, 0), jnp.clip(t, 0, NT)


def _kernel(x_h, wqkv_h, wo_h, wg_h, wu_h, wd_h, out_h,
            x_s, wqkv_v, wo_v, wg_v, wu_v, wd_v, opq, opk, opv, wo_e, wg_e, wu_e, wd_e,
            xa_s, q_s, k_s, v_s, o_s, out_s, zero_s, sems):

    def cp_x(t):
        return pltpu.make_async_copy(x_h.at[_ds(t, M), :], x_s.at[_ds(t, M), :], sems.at[SEM_X + t])

    def cp_w(p, rows, sem):
        return pltpu.make_async_copy(wqkv_h.at[:, rows, pl.ds(p * D, D)], wqkv_v.at[:, rows, pl.ds(p * D, D)],
                                     sems.at[sem])

    def cp_q(r):
        return cp_w(0, _ds(r, HD // QC), SEM_Q + r)

    def cp_kv(j):
        return [cp_w(p, _ds(j, HD // NT), SEM_KV + j) for p in (1, 2)]

    rest = [(wg_h, wg_v, wg_e, HD // NT, HF), (wu_h, wu_v, wu_e, HD // NT, HF), (wo_h, wo_v, wo_e, HD // NT, HD)]

    def cp_rest(j):
        return [pltpu.make_async_copy(src.at[:, _ds(j, n), :], raw.at[:, _ds(j, n), :], sems.at[SEM_REST + j])
                for src, raw, n in [(r[0], r[1], r[3]) for r in rest] + [(wd_h, wd_v, QF // NT)]]

    def layernorm(t):
        def norm(r0):
            x = x_s[pl.ds(pl.multiple_of(t * M + r0, LG), LG), :].astype(f32)
            xc = x - jnp.mean(x, axis=-1, keepdims=True)
            return xc * lax.rsqrt(jnp.mean(xc * xc, axis=-1, keepdims=True) + 1e-5)
        for r in range(0, HM, LG):
            top, bot = norm(r), norm(HM + r)
            a = _left(top[:, :HD], top[:, HD:], bot[:, :HD], bot[:, HD:])
            for i in range(7):
                xa_s[i, pl.ds(pl.multiple_of(t * (HM // 2) + r // 2, LG // 2), LG // 2), :] = pltpu.bitcast(a[i], i32)

    def load_a(i, t):
        return pltpu.bitcast(xa_s[i, _ds(t, HM // 2), :], bf16)

    def prep_part(p, op, r, n):
        rows, wrows = _ds(r, n), _ds(r, n // 2)
        blk = []
        for half in range(2):
            w = pltpu.bitcast(wqkv_v[half, rows, pl.ds(p * D, D)], i32)
            t = _twist([w[:, c * 128:(c + 1) * 128] for c in range(8)])
            blk += [jnp.concatenate(t[:4], axis=1), jnp.concatenate(t[4:], axis=1)]
        sums = _right_sums(*[pltpu.bitcast(b, bf16) for b in blk])
        for i, v in zip((0, 2, 3, 5, 6, 1, 4), sums + [blk[0], blk[3]]):
            op[i, wrows, :] = v

    def prep_rest(j):
        zero = zero_s[0]

        def through_xlu(b):
            return jnp.concatenate([pltpu.bitcast(pltpu.roll(pltpu.bitcast(b[:, k:k + 128], i32), zero, 1), bf16)
                                    for k in range(0, CB, 128)], axis=1)
        for _, raw, ext, n, hn in rest:
            for r in range(0, n, RB):
                rows = pl.ds(pl.multiple_of(j * n + r, RB), RB)
                wrows = pl.ds(pl.multiple_of((j * n + r) // 2, RB // 2), RB // 2)
                for c in range(0, hn, CB):
                    e = _right_sums(through_xlu(raw[0, rows, c:c + CB]), raw[0, rows, hn + c:hn + c + CB],
                                    raw[1, rows, c:c + CB], through_xlu(raw[1, rows, hn + c:hn + c + CB]))
                    for i in range(5):
                        ext[i, wrows, c:c + CB] = e[i]
        n = QF // NT
        for r in range(0, n, RB):
            rows = pl.ds(pl.multiple_of(j * n + r, RB), RB)
            wrows = pl.ds(pl.multiple_of((j * n + r) // 2, RB // 2), RB // 2)
            for c in range(0, QD, 128):
                def blk(ka, na):
                    return [pltpu.bitcast(pltpu.roll(pltpu.bitcast(
                        wd_v[2 * ka + kb, rows, na * HD + nb * QD + c:na * HD + nb * QD + c + 128], i32), zero, 1),
                        bf16).astype(f32) for kb in (0, 1) for nb in (0, 1)]
                level1 = zip(*[_right_f32(*p) for p in zip(blk(0, 0), blk(0, 1), blk(1, 0), blk(1, 1))])
                for i, r1 in enumerate(level1):
                    for k, v in enumerate(_right_f32(*r1)):
                        if (i, k) in SLOT2:
                            wd_e[SLOT2[i, k], wrows, c:c + 128] = pltpu.bitcast(v.astype(bf16), i32)

    def qkv_dot(t, op, dst, off):
        ts = _same(t)
        for n, n0 in enumerate(range(0, HD, NB)):
            c = _strassen(lambda i: _dot(load_a(i, ts[n % 4]), pltpu.bitcast(op[i, :, n0:n0 + NB], bf16)))
            for bi, blk in enumerate(c):
                dst[pl.ds(pl.multiple_of(t * M, M) + off + (bi // 2) * HM, HM),
                    (bi % 2) * HD + n0:(bi % 2) * HD + n0 + NB] = blk.astype(dst.dtype)

    def prologue():
        zero_s[0] = 0
        cp_x(0).start()
        for r in range(QC):
            cp_q(r).start()

        def start_kv(j, carry):
            @pl.when(j < NT - 1)
            def _():
                cp_x(jnp.minimum(j + 1, NT - 1)).start()
            for c in cp_kv(j):
                c.start()
            return carry
        lax.fori_loop(0, NT, start_kv, 0)

        def start_rest(j, carry):
            for c in cp_rest(j):
                c.start()
            return carry
        lax.fori_loop(0, NT, start_rest, 0)
        k_s[pl.ds(0, HALO), :] = jnp.zeros((HALO, D), f32)
        cp_x(0).wait()
        layernorm(0)

        def prep_q(r, carry):
            cp_q(r).wait()
            prep_part(0, opq, r, HD // QC)
            return carry
        lax.fori_loop(0, QC, prep_q, 0)

    def q_pass(j, carry):
        nxt = jnp.minimum(j + 1, NT - 1)

        @pl.when(j < NT - 1)
        def _():
            cp_x(nxt).wait()
        for c in cp_kv(j):
            c.wait()
        qkv_dot(j, opq, q_s, 0)
        prep_part(1, opk, j, HD // NT)
        prep_part(2, opv, j, HD // NT)
        layernorm(nxt)
        return carry

    def kv_pass(i, carry):
        for u in range(KVU):
            for c in cp_rest(KVU * i + u):
                c.wait()
        for u in range(KVU):
            j = KVU * i + u
            qkv_dot(j, opk, k_s, HALO)
            qkv_dot(jnp.minimum(j, NT - 1), opv, v_s, HALO)
            prep_rest(j)
        return carry

    def attention(base, r0):
        def taps(ref, m):
            kk = ref[pl.ds(base + r0, R + HALO), m * 128:(m + 1) * 128]
            out = [None] * W
            for r in range(4):
                a = kk[8 - DIL * r:8 - DIL * r + R + 8]
                out[r], out[r + 4] = a[8:R + 8], a[0:R]
            return out
        prods = [[] for _ in range(W)]
        for m in range(8):
            qm = q_s[pl.ds(base + r0, R), m * 128:(m + 1) * 128].astype(f32)
            km = taps(k_s, m)
            for w in range(W):
                prods[w].append(qm * km[w])
        lane = lax.broadcasted_iota(i32, (R, 128), 1)
        pos = base + r0 + lax.broadcasted_iota(i32, (R, 128), 0)
        logits = []
        for w in range(W):
            l = _tree_sum(prods[w])
            l = l + jnp.take_along_axis(l, lane ^ 1, axis=1)
            l = l + jnp.take_along_axis(l, lane ^ 2, axis=1)
            if w > 0:
                l = jnp.where(pos >= DIL * w, l, MASKED)
            logits.append(l)
        mx = functools.reduce(jnp.maximum, logits)
        es = [jnp.exp2((l - mx) * EXP_C) for l in logits]
        inv = 1.0 / _tree_sum(es)
        a = [e * inv for e in es]
        ot = []
        for m in range(8):
            vm = taps(v_s, m)
            ot.append(_tree_sum([a[w] * vm[w] for w in range(W)]))
        o_s[pl.ds(r0, R), :] = jnp.concatenate(_untwist(ot), axis=1)

    def out_copies(t):
        slot = t % 2
        return [pltpu.make_async_copy(
            out_s.at[slot, pl.ds(r0, HM), pl.ds(c0, HD)],
            out_h.at[pl.ds(pl.multiple_of(t * M + r0, HM), HM), pl.ds(c0, HD)], sems.at[SEM_OUT + slot])
            for r0 in (0, HM) for c0 in (0, HD)]

    def ffn_pass(t, carry):
        @pl.when(t >= 2)
        def _():
            for c in out_copies(t - 2):
                c.wait()
        base = pl.multiple_of(t * M, M)
        ts = _same(t)
        qm = HM // 2

        def hidden(c0, cn, n):
            out = []
            for sub in range(2):
                n0 = sub * QF + c0
                g = _combine([_dot(load_a(i, ts[(n + 2 * sub) % 4]), _right(wg_v, wg_e, i, HF, 0, HD, n0, cn))
                              for i in range(7)])
                u = _combine([_dot(load_a(i, ts[(n + 2 * sub + 1) % 4]), _right(wu_v, wu_e, i, HF, 0, HD, n0, cn))
                              for i in range(7)])
                out.append(_left_f32(*[_silu(g[i]) * u[i] for i in range(4)]))
            return out

        def wd_operand(i, k, c0, cn):
            if (i, k) in RAW2:
                kq, nq = RAW2[i, k]
                return wd_v[kq, c0:c0 + cn, nq * QD:(nq + 1) * QD]
            return pltpu.bitcast(wd_e[SLOT2[i, k], c0 // 2:(c0 + cn) // 2, :], bf16)

        def left2(e, i):
            return _left(e[0][i][:qm], e[1][i][:qm], e[0][i][qm:], e[1][i][qm:])

        es = [left2(e, i) for e in [hidden(c0, cn, n) for n, (c0, cn) in enumerate(FCHUNKS)] for i in range(7)]
        for r0 in range(0, M, R):
            attention(base, r0)
        part = {}
        for n, (c0, cn) in enumerate(FCHUNKS):
            for i in range(7):
                for k in range(7):
                    d = _dot(es[7 * n + i][k], wd_operand(i, k, c0, cn))
                    part[i, k] = d if n == 0 else part[i, k] + d
        md = []
        for i in range(7):
            c = _combine([part[i, k] for k in range(7)])
            md.append(jnp.concatenate([jnp.concatenate(c[:2], axis=1), jnp.concatenate(c[2:], axis=1)], axis=0))
        gate = [_silu(y) for y in _combine(md)]
        oa = _left(o_s[0:HM, 0:HD], o_s[0:HM, HD:D], o_s[HM:M, 0:HD], o_s[HM:M, HD:D])
        s = _strassen(lambda i: _dot(oa[i], _right(wo_v, wo_e, i, HD, 0, HD, 0, HD)))
        copies = out_copies(t)
        for bi in (2, 1, 0, 3):
            r0, c0 = (bi // 2) * HM, (bi % 2) * HD
            xr = x_s[pl.ds(base + r0, HM), c0:c0 + HD].astype(f32)
            out_s[t % 2, r0:r0 + HM, c0:c0 + HD] = (xr + s[bi] * gate[bi]).astype(bf16)
            copies[bi].start()
        return carry

    prologue()
    lax.fori_loop(0, NT, q_pass, 0)
    lax.fori_loop(0, NT // KVU, kv_pass, 0)
    v_s[pl.ds(0, HALO), :] = jnp.broadcast_to(v_s[pl.ds(HALO, 1), :], (HALO, D))
    lax.fori_loop(0, NT, ffn_pass, 0)
    for t in (NT - 2, NT - 1):
        for c in out_copies(t):
            c.wait()


@jax.jit
def pallas_recurrent_scan__sliding_local_dilated__swiglu_ffn__prompt_kernel(
    A_x: jax.Array,
    A_wqkv: jax.Array,
    A_wo: jax.Array,
    B_x: jax.Array,
    B_w_gate: jax.Array,
    B_w_up: jax.Array,
    B_w_down: jax.Array,
):
    del B_x
    out = pl.pallas_call(
        _kernel,
        in_specs=[pl.BlockSpec(memory_space=pl.ANY)] * 6,
        out_specs=pl.BlockSpec(memory_space=pl.ANY),
        out_shape=jax.ShapeDtypeStruct((S, D), bf16),
        scratch_shapes=[
            pltpu.VMEM((S, D), bf16),
            pltpu.VMEM((2, HD, 3 * D), bf16), pltpu.VMEM((2, HD, D), bf16),
            pltpu.VMEM((2, HD, F), bf16), pltpu.VMEM((2, HD, F), bf16), pltpu.VMEM((4, QF, D), bf16),
            pltpu.VMEM((7, HD // 2, HD), i32), pltpu.VMEM((7, HD // 2, HD), i32), pltpu.VMEM((7, HD // 2, HD), i32),
            pltpu.VMEM((5, HD // 2, HD), i32),
            pltpu.VMEM((5, HD // 2, HF), i32), pltpu.VMEM((5, HD // 2, HF), i32), pltpu.VMEM((len(SLOT2), QF // 2, QD), i32),
            pltpu.VMEM((7, S // 4, HD), i32),
            pltpu.VMEM((S, D), bf16), pltpu.VMEM((S + HALO, D), f32), pltpu.VMEM((S + HALO, D), f32),
            pltpu.VMEM((M, D), f32),
            pltpu.VMEM((2, M, D), bf16),
            pltpu.SMEM((1,), i32),
            pltpu.SemaphoreType.DMA((NSEM,)),
        ],
        compiler_params=pltpu.CompilerParams(
            vmem_limit_bytes=127 * 1024 * 1024,
            disable_semaphore_checks=True,
            flags={"XLA_TPU_EVENLY_DISTRIBUTE_CRITICAL_NODES": True},
        ),
    )(A_x.reshape(S, D), A_wqkv.reshape(2, HD, 3 * D), A_wo.reshape(2, HD, D), B_w_gate.reshape(2, HD, F),
      B_w_up.reshape(2, HD, F), B_w_down.reshape(4, QF, D))
    return out.reshape(1, S, D)
```

```python
import functools

import jax
from jax import lax
import jax.experimental.pallas as pl
import jax.experimental.pallas.tpu as pltpu
import jax.numpy as jnp
import numpy as np

S, D, F = 2048, 1024, 3584
DH, W, DIL = 32, 8, 2
HALO = 16
HD, HF, QD, QF = D // 2, F // 2, D // 4, F // 4
M = 256
HM = M // 2
NT = S // M
R = 16
LG = 16
NB = 128
FCHUNKS = ((0, 512), (512, 384))
CW = 128
KVU = 2
QC = 4
RB, CB = 16, 256
EXP_C = float(DH ** -0.5 * np.log2(np.e))
MASKED = float(-1e9 * DH ** 0.5)
SEM_X, SEM_Q, SEM_KV, SEM_REST, SEM_OUT = 0, NT, NT + QC, 2 * NT + QC, 3 * NT + QC
NSEM = 3 * NT + QC + 2

f32, bf16, i32 = jnp.float32, jnp.bfloat16, jnp.int32


def _twist_level(a, b, bit, lane):
    lo = (lane & (1 << bit)) == 0
    return jnp.where(lo, a, b), jnp.take_along_axis(jnp.where(lo, b, a), lane ^ (1 << bit), axis=1)


def _untwist_level(x, y, bit, lane):
    lo = (lane & (1 << bit)) == 0
    yp = jnp.take_along_axis(y, lane ^ (1 << bit), axis=1)
    return jnp.where(lo, x, yp), jnp.where(lo, yp, x)


def _twist(c):
    lane = lax.broadcasted_iota(i32, c[0].shape, 1)
    n = [None] * 8
    for p in range(4):
        n[p], n[4 + p] = _twist_level(c[2 * p], c[2 * p + 1], 4, lane)
    c, n = n, [None] * 8
    for g in range(0, 8, 4):
        for p in range(2):
            n[g + p], n[g + 2 + p] = _twist_level(c[g + 2 * p], c[g + 2 * p + 1], 3, lane)
    c, n = n, [None] * 8
    for g in range(0, 8, 2):
        n[g], n[g + 1] = _twist_level(c[g], c[g + 1], 2, lane)
    return n


def _untwist(c):
    lane = lax.broadcasted_iota(i32, c[0].shape, 1)
    n = [None] * 8
    for g in range(0, 8, 2):
        n[g], n[g + 1] = _untwist_level(c[g], c[g + 1], 2, lane)
    c, n = n, [None] * 8
    for g in range(0, 8, 4):
        for p in range(2):
            n[g + 2 * p], n[g + 2 * p + 1] = _untwist_level(c[g + p], c[g + 2 + p], 3, lane)
    c, n = n, [None] * 8
    for p in range(4):
        n[2 * p], n[2 * p + 1] = _untwist_level(c[p], c[4 + p], 4, lane)
    return n


def _dot(a, b):
    return jnp.dot(a, b, preferred_element_type=f32)


def _left_f32(a11, a12, a21, a22):
    return [a11 + a22, a21 + a22, a11, a22, a11 + a12, a21 - a11, a12 - a22]


def _left(*blocks):
    return [a.astype(bf16) for a in _left_f32(*blocks)]


def _right_sums(b11, b12, b21, b22):
    b11, b12, b21, b22 = [b.astype(f32) for b in (b11, b12, b21, b22)]
    return [pltpu.bitcast(v.astype(bf16), i32) for v in (b11 + b22, b12 - b22, b21 - b11, b11 + b12, b21 + b22)]


def _right_f32(b11, b12, b21, b22):
    return [b11 + b22, b11, b12 - b22, b21 - b11, b22, b11 + b12, b21 + b22]


RAW2 = {(1, 1): (0, 0), (1, 4): (1, 1), (4, 1): (2, 2), (4, 4): (3, 3)}
SLOT2 = {p: n for n, p in enumerate(p for p in ((i, k) for i in range(7) for k in range(7)) if p not in RAW2)}


def _right(raw, ext, i, hn, k0, kn, n0, nn):
    if i in (1, 4):
        r = 0 if i == 1 else 1
        return raw[r, k0:k0 + kn, r * hn + n0:r * hn + n0 + nn]
    e = {0: 0, 2: 1, 3: 2, 5: 3, 6: 4}[i]
    return pltpu.bitcast(ext[e, k0 // 2:(k0 + kn) // 2, n0:n0 + nn], bf16)


def _strassen(prod):
    m2, m4 = prod(1), prod(3)
    c21 = m2 + m4
    m3 = prod(2)
    c22 = m3 - m2
    m5 = prod(4)
    c12 = m3 + m5
    c11 = m4 - m5
    m1 = prod(0)
    c11 = c11 + m1 + prod(6)
    c22 = c22 + m1 + prod(5)
    return c11, c12, c21, c22


def _combine(m):
    return m[0] + m[3] - m[4] + m[6], m[2] + m[4], m[1] + m[3], m[0] - m[1] + m[2] + m[5]


def _tree_sum(xs):
    xs = list(xs)
    while len(xs) > 1:
        xs = [xs[i] + xs[i + 1] for i in range(0, len(xs), 2)]
    return xs[0]


def _silu(g):
    hg = 0.5 * g
    return hg * jnp.tanh(hg) + hg


def _ds(i, n):
    return pl.ds(pl.multiple_of(i * n, n), n)


def _same(t):
    return t, jnp.minimum(t, NT - 1), jnp.maximum(t, 0), jnp.clip(t, 0, NT)


def _kernel(x_h, wqkv_h, wo_h, wg_h, wu_h, wd_h, out_h,
            x_s, wqkv_v, wo_v, wg_v, wu_v, wd_v, opq, opk, opv, wo_e, wg_e, wu_e, wd_e,
            xa_s, xb_s, q_s, k_s, v_s, o_s, out_s, zero_s, sems):

    def cp_x(t):
        return pltpu.make_async_copy(x_h.at[_ds(t, M), :], x_s.at[_ds(t, M), :], sems.at[SEM_X + t])

    def cp_w(p, rows, sem):
        return pltpu.make_async_copy(wqkv_h.at[:, rows, pl.ds(p * D, D)], wqkv_v.at[:, rows, pl.ds(p * D, D)],
                                     sems.at[sem])

    def cp_q(r):
        return cp_w(0, _ds(r, HD // QC), SEM_Q + r)

    def cp_kv(j):
        return [cp_w(p, _ds(j, HD // NT), SEM_KV + j) for p in (1, 2)]

    rest = [(wg_h, wg_v, wg_e, HD // NT, HF), (wo_h, wo_v, wo_e, HD // NT, HD)]
    rest2 = [(wd_h, wd_v, wd_e, QF // NT, QD), (wu_h, wu_v, wu_e, QD // NT, QF)]

    def cp_rest(j):
        return [pltpu.make_async_copy(src.at[:, _ds(j, n), :], raw.at[:, _ds(j, n), :], sems.at[SEM_REST + j])
                for src, raw, _, n, _ in rest + rest2]

    def norm(t, r0):
        x = x_s[pl.ds(pl.multiple_of(t * M + r0, LG), LG), :].astype(f32)
        xc = x - jnp.mean(x, axis=-1, keepdims=True)
        return xc * lax.rsqrt(jnp.mean(xc * xc, axis=-1, keepdims=True) + 1e-5)

    def layernorm(t):
        for r in range(0, HM, LG):
            top, bot = norm(t, r), norm(t, HM + r)
            a = _left(top[:, :HD], top[:, HD:], bot[:, :HD], bot[:, HD:])
            for i in range(7):
                xa_s[i, pl.ds(pl.multiple_of(t * (HM // 2) + r // 2, LG // 2), LG // 2), :] = pltpu.bitcast(a[i], i32)

    def layernorm2(t):
        qm = HM // 2
        for r in range(0, qm, LG):
            rows = [pl.ds(pl.multiple_of(t * M + rq * qm + r, LG), LG) for rq in range(4)]
            stats = []
            for rw in rows:
                x = x_s[rw, :].astype(f32)
                mu = jnp.mean(x, axis=-1, keepdims=True)
                stats.append((mu, lax.rsqrt(jnp.mean((x - mu) * (x - mu), axis=-1, keepdims=True) + 1e-5)))
            for c in range(0, QD, CW):
                def blk(ra, ca):
                    return [(x_s[rows[2 * ra + rb], (2 * ca + cb) * QD + c:(2 * ca + cb) * QD + c + CW].astype(f32)
                             - stats[2 * ra + rb][0]) * stats[2 * ra + rb][1] for rb in (0, 1) for cb in (0, 1)]
                level1 = zip(*[_left_f32(*p) for p in zip(blk(0, 0), blk(0, 1), blk(1, 0), blk(1, 1))])
                for i, a1 in enumerate(level1):
                    for k, a in enumerate(_left(*a1)):
                        xb_s[7 * i + k, r // 2:(r + LG) // 2, c:c + CW] = pltpu.bitcast(a, i32)

    def load_a(i, t):
        return pltpu.bitcast(xa_s[i, _ds(t, HM // 2), :], bf16)

    def prep_part(p, op, r, n):
        rows, wrows = _ds(r, n), _ds(r, n // 2)
        blk = []
        for half in range(2):
            w = pltpu.bitcast(wqkv_v[half, rows, pl.ds(p * D, D)], i32)
            t = _twist([w[:, c * 128:(c + 1) * 128] for c in range(8)])
            blk += [jnp.concatenate(t[:4], axis=1), jnp.concatenate(t[4:], axis=1)]
        sums = _right_sums(*[pltpu.bitcast(b, bf16) for b in blk])
        for i, v in zip((0, 2, 3, 5, 6, 1, 4), sums + [blk[0], blk[3]]):
            op[i, wrows, :] = v

    def prep_rest(j):
        zero = zero_s[0]

        def through_xlu(b):
            return jnp.concatenate([pltpu.bitcast(pltpu.roll(pltpu.bitcast(b[:, k:k + 128], i32), zero, 1), bf16)
                                    for k in range(0, CB, 128)], axis=1)
        for _, raw, ext, n, hn in rest:
            for r in range(0, n, RB):
                rows = pl.ds(pl.multiple_of(j * n + r, RB), RB)
                wrows = pl.ds(pl.multiple_of((j * n + r) // 2, RB // 2), RB // 2)
                for c in range(0, hn, CB):
                    e = _right_sums(through_xlu(raw[0, rows, c:c + CB]), raw[0, rows, hn + c:hn + c + CB],
                                    raw[1, rows, c:c + CB], through_xlu(raw[1, rows, hn + c:hn + c + CB]))
                    for i in range(5):
                        ext[i, wrows, c:c + CB] = e[i]
        for _, raw, ext, n, qn in rest2:
            for r in range(0, n, RB):
                rows = pl.ds(pl.multiple_of(j * n + r, RB), RB)
                wrows = pl.ds(pl.multiple_of((j * n + r) // 2, RB // 2), RB // 2)
                for c in range(0, qn, 128):
                    def blk(ka, na):
                        return [pltpu.bitcast(pltpu.roll(pltpu.bitcast(
                            raw[2 * ka + kb, rows, (2 * na + nb) * qn + c:(2 * na + nb) * qn + c + 128], i32), zero, 1),
                            bf16).astype(f32) for kb in (0, 1) for nb in (0, 1)]
                    level1 = zip(*[_right_f32(*p) for p in zip(blk(0, 0), blk(0, 1), blk(1, 0), blk(1, 1))])
                    for i, r1 in enumerate(level1):
                        for k, v in enumerate(_right_f32(*r1)):
                            if (i, k) in SLOT2:
                                ext[SLOT2[i, k], wrows, c:c + 128] = pltpu.bitcast(v.astype(bf16), i32)

    def qkv_dot(t, op, dst, off):
        ts = _same(t)
        for n, n0 in enumerate(range(0, HD, NB)):
            c = _strassen(lambda i: _dot(load_a(i, ts[n % 4]), pltpu.bitcast(op[i, :, n0:n0 + NB], bf16)))
            for bi, blk in enumerate(c):
                dst[pl.ds(pl.multiple_of(t * M, M) + off + (bi // 2) * HM, HM),
                    (bi % 2) * HD + n0:(bi % 2) * HD + n0 + NB] = blk.astype(dst.dtype)

    def prologue():
        zero_s[0] = 0
        cp_x(0).start()
        for r in range(QC):
            cp_q(r).start()

        def start_kv(j, carry):
            @pl.when(j < NT - 1)
            def _():
                cp_x(jnp.minimum(j + 1, NT - 1)).start()
            for c in cp_kv(j):
                c.start()
            return carry
        lax.fori_loop(0, NT, start_kv, 0)

        def start_rest(j, carry):
            for c in cp_rest(j):
                c.start()
            return carry
        lax.fori_loop(0, NT, start_rest, 0)
        k_s[pl.ds(0, HALO), :] = jnp.zeros((HALO, D), bf16)
        cp_x(0).wait()
        layernorm(0)

        def prep_q(r, carry):
            cp_q(r).wait()
            prep_part(0, opq, r, HD // QC)
            return carry
        lax.fori_loop(0, QC, prep_q, 0)
        layernorm2(0)

    def q_pass(j, carry):
        nxt = jnp.minimum(j + 1, NT - 1)

        @pl.when(j < NT - 1)
        def _():
            cp_x(nxt).wait()
        for c in cp_kv(j):
            c.wait()
        qkv_dot(j, opq, q_s, 0)
        prep_part(1, opk, j, HD // NT)
        prep_part(2, opv, j, HD // NT)
        layernorm(nxt)
        return carry

    def kv_pass(i, carry):
        for u in range(KVU):
            for c in cp_rest(KVU * i + u):
                c.wait()
        for u in range(KVU):
            j = KVU * i + u
            qkv_dot(j, opk, k_s, HALO)
            qkv_dot(jnp.minimum(j, NT - 1), opv, v_s, HALO)
            prep_rest(j)
        return carry

    def attention(base, r0):
        def taps(ref, m):
            kk = ref[pl.ds(base + r0, R + HALO), m * 128:(m + 1) * 128].astype(f32)
            out = [None] * W
            for r in range(4):
                a = kk[8 - DIL * r:8 - DIL * r + R + 8]
                out[r], out[r + 4] = a[8:R + 8], a[0:R]
            return out
        prods = [[] for _ in range(W)]
        for m in range(8):
            qm = q_s[pl.ds(base + r0, R), m * 128:(m + 1) * 128].astype(f32)
            km = taps(k_s, m)
            for w in range(W):
                prods[w].append(qm * km[w])
        lane = lax.broadcasted_iota(i32, (R, 128), 1)
        pos = base + r0 + lax.broadcasted_iota(i32, (R, 128), 0)
        logits = []
        for w in range(W):
            l = _tree_sum(prods[w])
            l = l + jnp.take_along_axis(l, lane ^ 1, axis=1)
            l = l + jnp.take_along_axis(l, lane ^ 2, axis=1)
            if w > 0:
                l = jnp.where(pos >= DIL * w, l, MASKED)
            logits.append(l)
        mx = functools.reduce(jnp.maximum, logits)
        es = [jnp.exp2((l - mx) * EXP_C) for l in logits]
        inv = 1.0 / _tree_sum(es)
        a = [e * inv for e in es]
        ot = []
        for m in range(8):
            vm = taps(v_s, m)
            ot.append(_tree_sum([a[w] * vm[w] for w in range(W)]))
        o_s[pl.ds(r0, R), :] = jnp.concatenate(_untwist(ot), axis=1)

    def out_copies(t):
        slot = t % 2
        return [pltpu.make_async_copy(
            out_s.at[slot, pl.ds(r0, HM), pl.ds(c0, HD)],
            out_h.at[pl.ds(pl.multiple_of(t * M + r0, HM), HM), pl.ds(c0, HD)], sems.at[SEM_OUT + slot])
            for r0 in (0, HM) for c0 in (0, HD)]

    def ffn_pass(t, carry):
        @pl.when(t >= 2)
        def _():
            for c in out_copies(t - 2):
                c.wait()
        base = pl.multiple_of(t * M, M)
        ts = _same(t)
        qm = HM // 2

        def hidden(c0, cn, n):
            def wu_operand(i, k):
                if (i, k) in RAW2:
                    kq, nq = RAW2[i, k]
                    return wu_v[kq, :, nq * QF + c0:nq * QF + c0 + cn]
                return pltpu.bitcast(wu_e[SLOT2[i, k], :, c0:c0 + cn], bf16)
            mu = [_strassen(lambda k: _dot(pltpu.bitcast(xb_s[7 * i + k], bf16), wu_operand(i, k))) for i in range(7)]
            out = []
            for sub in range(2):
                g = _combine([_dot(load_a(i, ts[(2 * n + sub) % 4]), _right(wg_v, wg_e, i, HF, 0, HD, sub * QF + c0, cn))
                              for i in range(7)])
                u = _combine([jnp.concatenate([c[sub], c[2 + sub]], axis=0) for c in mu])
                out.append(_left_f32(*[_silu(g[i]) * u[i] for i in range(4)]))
            return out

        def wd_operand(i, k, c0, cn):
            if (i, k) in RAW2:
                kq, nq = RAW2[i, k]
                return wd_v[kq, c0:c0 + cn, nq * QD:(nq + 1) * QD]
            return pltpu.bitcast(wd_e[SLOT2[i, k], c0 // 2:(c0 + cn) // 2, :], bf16)

        def left2(e, i):
            return _left(e[0][i][:qm], e[1][i][:qm], e[0][i][qm:], e[1][i][qm:])

        es = [left2(e, i) for e in [hidden(c0, cn, n) for n, (c0, cn) in enumerate(FCHUNKS)] for i in range(7)]
        layernorm2(jnp.minimum(t + 1, NT - 1))
        for r0 in range(0, M, R):
            attention(base, r0)
        part = {}
        for n, (c0, cn) in enumerate(FCHUNKS):
            for i in range(7):
                for k in range(7):
                    d = _dot(es[7 * n + i][k], wd_operand(i, k, c0, cn))
                    part[i, k] = d if n == 0 else part[i, k] + d
        md = []
        for i in range(7):
            c = _combine([part[i, k] for k in range(7)])
            md.append(jnp.concatenate([jnp.concatenate(c[:2], axis=1), jnp.concatenate(c[2:], axis=1)], axis=0))
        gate = [_silu(y) for y in _combine(md)]
        oa = _left(o_s[0:HM, 0:HD], o_s[0:HM, HD:D], o_s[HM:M, 0:HD], o_s[HM:M, HD:D])
        s = _strassen(lambda i: _dot(oa[i], _right(wo_v, wo_e, i, HD, 0, HD, 0, HD)))
        copies = out_copies(t)
        for bi in (2, 1, 0, 3):
            r0, c0 = (bi // 2) * HM, (bi % 2) * HD
            xr = x_s[pl.ds(base + r0, HM), c0:c0 + HD].astype(f32)
            out_s[t % 2, r0:r0 + HM, c0:c0 + HD] = (xr + s[bi] * gate[bi]).astype(bf16)
            copies[bi].start()
        return carry

    prologue()
    lax.fori_loop(0, NT, q_pass, 0)
    lax.fori_loop(0, NT // KVU, kv_pass, 0)
    v_s[pl.ds(0, HALO), :] = jnp.broadcast_to(v_s[pl.ds(HALO, HALO), :].astype(f32)[0:1], (HALO, D)).astype(bf16)
    lax.fori_loop(0, NT, ffn_pass, 0)
    for t in (NT - 2, NT - 1):
        for c in out_copies(t):
            c.wait()


@jax.jit
def pallas_recurrent_scan__sliding_local_dilated__swiglu_ffn__prompt_kernel(
    A_x: jax.Array,
    A_wqkv: jax.Array,
    A_wo: jax.Array,
    B_x: jax.Array,
    B_w_gate: jax.Array,
    B_w_up: jax.Array,
    B_w_down: jax.Array,
):
    del B_x
    out = pl.pallas_call(
        _kernel,
        in_specs=[pl.BlockSpec(memory_space=pl.ANY)] * 6,
        out_specs=pl.BlockSpec(memory_space=pl.ANY),
        out_shape=jax.ShapeDtypeStruct((S, D), bf16),
        scratch_shapes=[
            pltpu.VMEM((S, D), bf16),
            pltpu.VMEM((2, HD, 3 * D), bf16), pltpu.VMEM((2, HD, D), bf16),
            pltpu.VMEM((2, HD, F), bf16), pltpu.VMEM((4, QD, F), bf16), pltpu.VMEM((4, QF, D), bf16),
            pltpu.VMEM((7, HD // 2, HD), i32), pltpu.VMEM((7, HD // 2, HD), i32), pltpu.VMEM((7, HD // 2, HD), i32),
            pltpu.VMEM((5, HD // 2, HD), i32),
            pltpu.VMEM((5, HD // 2, HF), i32), pltpu.VMEM((len(SLOT2), QD // 2, QF), i32), pltpu.VMEM((len(SLOT2), QF // 2, QD), i32),
            pltpu.VMEM((7, S // 4, HD), i32),
            pltpu.VMEM((49, HM // 4, QD), i32),
            pltpu.VMEM((S, D), bf16), pltpu.VMEM((S + HALO, D), bf16), pltpu.VMEM((S + HALO, D), bf16),
            pltpu.VMEM((M, D), f32),
            pltpu.VMEM((2, M, D), bf16),
            pltpu.SMEM((1,), i32),
            pltpu.SemaphoreType.DMA((NSEM,)),
        ],
        compiler_params=pltpu.CompilerParams(
            vmem_limit_bytes=127 * 1024 * 1024,
            disable_semaphore_checks=True,
            flags={"XLA_TPU_EVENLY_DISTRIBUTE_CRITICAL_NODES": True},
        ),
    )(A_x.reshape(S, D), A_wqkv.reshape(2, HD, 3 * D), A_wo.reshape(2, HD, D), B_w_gate.reshape(2, HD, F),
      B_w_up.reshape(4, QD, F), B_w_down.reshape(4, QF, D))
    return out.reshape(1, S, D)
```
